```python
import os as _os
_os.environ.setdefault("JAX_PLATFORMS", "cpu")
import jax
import jax.numpy as jnp

def _softmax(x, axis=-1):
    return jax.nn.softmax(x, axis=axis)
def _gelu(x):
    return jax.nn.gelu(x, approximate=True)
def _silu(x):
    return jax.nn.silu(x)
def _sigmoid(x):
    return jax.nn.sigmoid(x)
def _layernorm(x, axis=-1, eps=1e-5):
    m = jnp.mean(x, axis=axis, keepdims=True)
    v = jnp.var(x, axis=axis, keepdims=True)
    return (x - m) / jnp.sqrt(v + eps)
def _scatter_add(tgt, idx, src, axis=0):
    return tgt.at[idx].add(src)
def _segment_sum(src, seg, n):
    return jax.ops.segment_sum(src, seg, n)
class _Rng:
    def __init__(self, key):
        self._k = key
    def _next(self):
        self._k, sub = jax.random.split(self._k)
        return sub
    def normal(self, shape):
        return jax.random.normal(self._next(), shape, dtype=jnp.bfloat16)
    def randint(self, lo, hi, shape):
        return jax.random.randint(self._next(), shape, lo, hi, dtype=jnp.int32)
    def uniform(self, shape, lo=0.0, hi=1.0):
        return jax.random.uniform(self._next(), shape, jnp.bfloat16, lo, hi)
    def permutation(self, n):
        return jax.random.permutation(self._next(), n)


kernel_name = 'gated_mix__ssm_conv_h3__linear_kernel_hedgehog__prompt'

def setup_inputs():
    _rng = _Rng(jax.random.key(int.from_bytes(__import__("os").urandom(4), "little")))
    _w = (lambda a: (lambda t: t.astype(jnp.bfloat16) if jnp.issubdtype(t.dtype, jnp.floating) else t)(jnp.asarray(a)))
    def _A_setup():
        B, S, D = 1, 2048, 576
        ks = 4
        return {
            "q": _w((lambda *s: _rng.normal(s) * 0.05)(B, S, D)),
            "k": _w((lambda *s: _rng.normal(s) * 0.4)(B, S, D)),
            "v": _w((lambda *s: _rng.normal(s) * 0.4)(B, S, D)),
            "shift_k": _w((lambda *s: _rng.normal(s) * 0.4)(D, ks) * 0.5),
            "ssm_k": _w((lambda *s: _rng.normal(s) * 0.4)(D, S) * (1.0 / S ** 0.5)),
            "ssm_D": _w((lambda *s: _rng.normal(s) * 0.4)(D)),
        }
    _A_in = _A_setup()

    def _B_setup():
        B, S, D, H = 1, 2048, 576, 32
        Dh = D // H
        return {
            "x": _w((lambda *s: _rng.normal(s) * 0.05)(B, S, D)),
            "wqkv": _w((lambda *s: _rng.normal(s) * 0.8)(D, 3 * D)),
            "w_phi": _w((lambda *s: _rng.normal(s) * 0.8)(H, Dh, Dh) * (Dh ** -0.5)),
            "wo": _w((lambda *s: _rng.normal(s) * 0.05)(D, D)),
        }
    _B_in = _B_setup()

    return {
        "A_q": _A_in["q"],
        "A_k": _A_in["k"],
        "A_v": _A_in["v"],
        "A_shift_k": _A_in["shift_k"],
        "A_ssm_k": _A_in["ssm_k"],
        "A_ssm_D": _A_in["ssm_D"],
        "B_x": _B_in["x"],
        "B_wqkv": _B_in["wqkv"],
        "B_w_phi": _B_in["w_phi"],
        "B_wo": _B_in["wo"],
        "gate_w": _w((lambda *s: _rng.normal(s) * 0.05)(576) * 16.0),
    }

def reference(A_q, A_k, A_v, A_shift_k, A_ssm_k, A_ssm_D, B_x, B_wqkv, B_w_phi, B_wo, gate_w):
    def _A_ref(q, k, v, shift_k, ssm_k, ssm_D):
        B, S, D = q.shape
        ks = shift_k.shape[-1]
        k_pad = jnp.pad(k, ((0, 0), (ks - 1, 0), (0, 0)))
        k_shift = jnp.zeros_like(k)
        for t in range(ks):
            k_shift = k_shift + k_pad[:, t:t + S, :] * shift_k[:, ks - 1 - t][None, None, :]
        kv = k_shift * v
        L = 2 * S
        kv_pad = jnp.pad(kv, ((0, 0), (0, S), (0, 0)))
        kf_pad = jnp.pad(ssm_k, ((0, 0), (0, S)))
        kv_f = (lambda x, axes=(-2,-1): jnp.fft.rfft2(x.astype(jnp.float32), axes=axes))(kv_pad[:, None, :, :], axes=(1, 2))
        kf_f = (lambda x, axes=(-2,-1): jnp.fft.rfft2(x.astype(jnp.float32), axes=axes))(kf_pad[:, None, :], axes=(1, 2))
        kf_f = (lambda x, *d: x.transpose(*d))(kf_f, 1, 2, 0)
        y_f = kv_f * kf_f[None, :, :, :]
        y = (lambda x, s, axes=(-2,-1): jnp.fft.irfft2(x, s=s, axes=axes).astype(jnp.bfloat16))(y_f, (1, L), axes=(1, 2))[:, 0, :S, :]
        y = y + kv * ssm_D[None, None, :]
        return q * y

    def _B_ref(x, wqkv, w_phi, wo):
        B, S, D = x.shape
        H = 32; Dh = D // H
        qkv = (lambda x, *d: x.transpose(*d))((x @ wqkv).reshape(B, S, 3, H, Dh), 2, 0, 3, 1, 4)
        q, k, v = qkv[0], qkv[1], qkv[2]
        pq = jnp.einsum("bhsd,hdf->bhsf", q, w_phi)
        pk = jnp.einsum("bhsd,hdf->bhsf", k, w_phi)
        phi_q = jnp.concatenate([_softmax(pq, axis=-1), _softmax(-pq, axis=-1)], axis=-1)
        phi_k = jnp.concatenate([_softmax(pk, axis=-1), _softmax(-pk, axis=-1)], axis=-1)
        kv = jnp.einsum("bhsf,bhsd->bhfd", phi_k, v)
        z  = jnp.einsum("bhsf->bhf", phi_k)
        num = jnp.einsum("bhqf,bhfd->bhqd", phi_q, kv)
        den = jnp.einsum("bhqf,bhf->bhq", phi_q, z)[..., None] + 1e-6
        o = num / den
        return (lambda x, *d: x.transpose(*d))(o, 0, 2, 1, 3).reshape(B, S, D) @ wo

    x = A_q
    g = _sigmoid((x * gate_w).sum(-1, keepdims=True))
    a = _A_ref(x, A_k, A_v, A_shift_k, A_ssm_k, A_ssm_D)
    b = _B_ref(x, B_wqkv, B_w_phi, B_wo)
    return g * a + (1 - g) * b
```

```python
import functools
import math

import jax
import jax.numpy as jnp
import numpy as np
import jax.experimental.pallas as pl
import jax.experimental.pallas.tpu as pltpu

S = 2048
D = 576
H = 32
DH = 18
NG = 4
GR = 144
B = 128
NB = S // B
NIT = 4
CC = D // NIT
SC = S // NIT
NT = SC // 128
MR = 3 * D + 16
KO, VO, QO, GO = 0, D, 2 * D, 3 * D
LOG2E = math.log2(math.e)
F32 = jnp.float32
BF16 = jnp.bfloat16
U32 = jnp.uint32


def _dft_consts():
    n = np.arange(B, dtype=np.float64)[:, None]
    k = np.arange(B, dtype=np.float64)[None, :]
    ang = 2.0 * np.pi * (2.0 * k + 0.5) * n / (2 * B)
    f = np.concatenate([np.cos(ang), -np.sin(ang)], axis=1)
    g = f.T / B
    return f.astype(np.float32), g.astype(np.float32)


def _nn(a, b):
    return jnp.dot(a, b, preferred_element_type=F32)


def _nt(a, b):
    return jax.lax.dot_general(a, b, (((1,), (1,)), ((), ())), preferred_element_type=F32)


def _pk(x):
    return pltpu.bitcast(x, U32)


def _up(x):
    return pltpu.bitcast(x, BF16)


def _kernel(x_hbm, k_hbm, v_hbm, sk_hbm, h_hbm, sd_hbm, w_hbm, wp_hbm, wo_hbm, gw_hbm, f_hbm, g_hbm,
            o_hbm,
            xb, kb, vb, hb, wb, wob, skb, sdb, gwb, wpb, fb, gb,
            wt, wot, cb, us, hs, ys, kvs, at, rs, phis, vts, pq, gs, kva, za, kvm, ob,
            sems, osems):
    def small(i, src, dst):
        return pltpu.make_async_copy(src, dst, sems.at[i])
    c_wp = small(0, wp_hbm, wpb)
    c_sk = small(1, sk_hbm, skb)
    c_sd = small(2, sd_hbm, sdb)
    c_gw = small(3, gw_hbm, gwb)
    c_f = small(4, f_hbm, fb)
    c_g = small(5, g_hbm, gb)
    c_w = small(6, w_hbm, wb)
    c_wo = small(7, wo_hbm, wob)

    def rows(src, dst, base, i):
        return pltpu.make_async_copy(src.at[pl.ds(i * CC, CC), :], dst.at[pl.ds(i * CC, CC), :], sems.at[base + i])

    def cols(i):
        return pltpu.make_async_copy(x_hbm.at[:, pl.ds(i * SC, SC)], xb.at[:, pl.ds(i * SC, SC)], sems.at[8 + i])

    for c in (c_wp, c_sk, c_sd, c_gw, c_f, c_g, c_w):
        c.start()
    for i in range(NIT):
        rows(h_hbm, hb, 12, i).start()
        rows(k_hbm, kb, 16, i).start()
        rows(v_hbm, vb, 20, i).start()
        if i == 0:
            for j in range(NIT):
                cols(j).start()
    c_wo.start()

    c_wp.wait(); c_sk.wait(); c_sd.wait(); c_gw.wait(); c_f.wait(); c_g.wait()

    hh = jax.lax.broadcasted_iota(jnp.int32, (H, 640), 0)
    cc = jax.lax.broadcasted_iota(jnp.int32, (H, 640), 1)
    amat = None
    for d in range(DH):
        e = jnp.where(cc == DH * hh + d, 1.0, 0.0).astype(BF16)
        t = _nn(wpb[d], e)
        amat = t if amat is None else amat + t
    amat_k = pltpu.roll(amat, 64, 1)

    skf = skb[...].astype(F32)
    for t in range(4):
        cb[t] = jnp.broadcast_to(skf[t:t + 1, :], (128, D)).T
    cb[4] = jnp.broadcast_to(sdb[...].astype(F32).reshape(1, D), (128, D)).T
    wt[GO // 2:GO // 2 + 8, :] = _pk(jnp.broadcast_to(gwb[...].astype(F32).reshape(1, D), (16, D)).astype(BF16))

    kva[...] = jnp.zeros(kva.shape, F32)
    za[...] = jnp.zeros(za.shape, F32)

    c_w.wait()
    h8 = jax.lax.broadcasted_iota(jnp.int32, (8, 256), 0)
    c8 = jax.lax.broadcasted_iota(jnp.int32, (8, 256), 1)
    for (am, off, t0, ro) in ((amat_k, 64, 4, KO), (amat, 0, 0, QO)):
        for g in range(NG):
            lo = DH * (8 * g + h8) + off - 128 * g
            msk = jnp.logical_and(c8 >= lo, c8 < lo + DH)
            aw = am[:, 128 * g:128 * g + 256]
            p = jnp.concatenate(
                [jnp.where(msk, jnp.broadcast_to(aw[f:f + 1, :], (8, 256)), 0.0) for f in range(DH)], axis=0)
            wf = _nt(p.astype(BF16), wb[:, 128 * (t0 + g):128 * (t0 + g) + 256]) * LOG2E
            r0 = (ro + g * GR) // 2
            wt[r0:r0 + GR // 2, :] = _pk(wf.astype(BF16))
    wt[VO // 2:(VO + D) // 2, :] = _pk(wb[:, 2 * D:3 * D].astype(F32).T.astype(BF16))

    lane = jax.lax.broadcasted_iota(jnp.int32, (8, 128), 1)

    def phase1(it, carry):
        c0 = pl.multiple_of(it * CC, 16)
        s0 = pl.multiple_of(it * SC, 128)
        rows(h_hbm, hb, 12, it).wait()
        rows(k_hbm, kb, 16, it).wait()
        rows(v_hbm, vb, 20, it).wait()

        @pl.when(it == 0)
        def _():
            for j in range(NIT):
                cols(j).wait()

        fmat = fb[...]
        hl = jnp.concatenate([hb[pl.ds(c0, CC), m * B:(m + 1) * B] for m in range(NB)], axis=0)
        hr = _nn(hl, fmat)
        for m in range(NB):
            cur = hr[m * CC:(m + 1) * CC]
            if m == 0:
                hs[0] = cur
            else:
                prv = hr[(m - 1) * CC:m * CC]
                hs[m, :, 0:B] = cur[:, 0:B] - prv[:, B:2 * B]
                hs[m, :, B:2 * B] = cur[:, B:2 * B] + prv[:, 0:B]
        for rg in range(CC // 8):
            r = pl.multiple_of(c0 + rg * 8, 8)
            co = [cb[t, pl.ds(r, 8), :] for t in range(4)]
            kf = kb[pl.ds(r, 8), :].astype(F32)
            vf = vb[pl.ds(r, 8), :].astype(F32)
            p1 = jnp.zeros((8, 128), F32)
            p2 = jnp.zeros((8, 128), F32)
            outs = []
            for j in range(NB):
                kj = kf[:, j * B:(j + 1) * B]
                r1 = pltpu.roll(kj, 1, 1)
                k1 = jnp.where(lane < 1, p1, r1)
                p1 = r1
                a = co[0] * kj + co[1] * k1
                b = co[2] * kj + co[3] * k1
                r2 = pltpu.roll(b, 2, 1)
                b2 = jnp.where(lane < 2, p2, r2)
                p2 = r2
                outs.append((a + b2) * vf[:, j * B:(j + 1) * B])
            kvs[rg * 64:(rg + 1) * 64, :] = _pk(jnp.concatenate(outs, axis=0).astype(BF16))
        ur = _nn(_up(kvs[...]), fmat)
        us[...] = ur
        rr = _nn(_up(wt[:, 512:D]), xb[512:D, pl.ds(s0, SC)])
        rs[...] = rr
        for n in range(NT):
            sn = pl.multiple_of(s0 + n * 128, 128)
            pr = _nn(_up(wt[:, 0:512]), xb[0:512, pl.ds(sn, 128)]) + rs[:, n * 128:(n + 1) * 128]
            for g in range(NG):
                p = [pr[KO + g * GR + f * 8:KO + g * GR + f * 8 + 8] for f in range(DH)]
                mx = functools.reduce(jnp.maximum, p)
                mn = functools.reduce(jnp.minimum, p)
                ep = [jnp.exp2(t - mx) for t in p]
                en = [jnp.exp2(mn - t) for t in p]
                rp = 1.0 / functools.reduce(jnp.add, ep)
                rn = 1.0 / functools.reduce(jnp.add, en)
                ph = jnp.concatenate([t * rp for t in ep] + [t * rn for t in en], axis=0)
                za[g * 288:(g + 1) * 288, :] += ph
                phis[g * 144:(g + 1) * 144, n * 128:(n + 1) * 128] = _pk(ph.astype(BF16))
            vts[:, n * 128:(n + 1) * 128] = _pk(pr[VO:VO + D].astype(BF16))
            pq[:, pl.ds(sn, 128)] = pr[QO:QO + D]
            gs[:, pl.ds(sn, 128)] = jax.nn.sigmoid(pr[GO:GO + 8])
        for g in range(NG):
            kva[g] += _nt(_up(vts[g * 72:(g + 1) * 72, :]), _up(phis[g * 144:(g + 1) * 144, :]))
        for rg in range(CC // 8):
            for i0 in range(0, NB, 4):
                acc = [None] * 4
                win = {}
                for j in range(i0 + 4):
                    u_re = us[rg * 128 + j * 8:rg * 128 + j * 8 + 8, 0:B]
                    u_im = us[rg * 128 + j * 8:rg * 128 + j * 8 + 8, B:2 * B]
                    for a in range(4):
                        m = i0 + a - j
                        if m < 0:
                            continue
                        if m not in win:
                            win[m] = (hs[m, rg * 8:rg * 8 + 8, 0:B], hs[m, rg * 8:rg * 8 + 8, B:2 * B])
                        h_re, h_im = win[m]
                        t_re = h_re * u_re - h_im * u_im
                        t_im = h_re * u_im + h_im * u_re
                        acc[a] = (t_re, t_im) if acc[a] is None else (acc[a][0] + t_re, acc[a][1] + t_im)
                r0 = rg * 64 + i0 * 4
                ys[r0:r0 + 16, 0:B] = _pk(jnp.concatenate([t[0] for t in acc], axis=0).astype(BF16))
                ys[r0:r0 + 16, B:2 * B] = _pk(jnp.concatenate([t[1] for t in acc], axis=0).astype(BF16))
        yr = _nn(_up(ys[...]), gb[...])
        for rg in range(CC // 8):
            r = pl.multiple_of(c0 + rg * 8, 8)
            dd = cb[4, pl.ds(r, 8), :]
            kvf = _up(kvs[rg * 64:(rg + 1) * 64, :]).astype(F32)
            qf = xb[pl.ds(r, 8), :].astype(F32)
            for i in range(NB):
                y = yr[rg * 128 + i * 8:rg * 128 + i * 8 + 8] + kvf[i * 8:i * 8 + 8] * dd
                at[pl.ds(r, 8), i * B:(i + 1) * B] = y * qf[:, i * B:(i + 1) * B]
        return carry

    jax.lax.fori_loop(0, NIT, phase1, 0)

    c_wo.wait()
    wot[...] = _pk(wob[...].astype(F32).T.astype(BF16))
    rh = jax.lax.broadcasted_iota(jnp.int32, (GR, 288), 0)
    ch = jax.lax.broadcasted_iota(jnp.int32, (GR, 288), 1) % 8
    kmask = jnp.logical_and(rh >= DH * ch, rh < DH * ch + DH)
    for g in range(NG):
        kvm[g] = _pk(jnp.where(kmask, kva[g], 0.0).astype(BF16))
    za[...] = jnp.broadcast_to(jnp.sum(za[...], axis=1, keepdims=True), za.shape)

    def out_copy(i):
        return pltpu.make_async_copy(ob.at[:, pl.ds(i * SC, SC)], o_hbm.at[:, pl.ds(i * SC, SC)], osems.at[i])

    def phase2(it, carry):
        s0 = pl.multiple_of(it * SC, 128)
        for n in range(NT):
            sn = pl.multiple_of(s0 + n * 128, 128)
            os_ = []
            for g in range(NG):
                p = [pq[g * GR + f * 8:g * GR + f * 8 + 8, pl.ds(sn, 128)] for f in range(DH)]
                mx = functools.reduce(jnp.maximum, p)
                mn = functools.reduce(jnp.minimum, p)
                ep = [jnp.exp2(t - mx) for t in p]
                en = [jnp.exp2(mn - t) for t in p]
                rp = 1.0 / functools.reduce(jnp.add, ep)
                rn = 1.0 / functools.reduce(jnp.add, en)
                dp = functools.reduce(jnp.add, [ep[f] * za[g * 288 + f * 8:g * 288 + f * 8 + 8, :] for f in range(DH)])
                dn = functools.reduce(jnp.add, [en[f] * za[g * 288 + 144 + f * 8:g * 288 + 144 + f * 8 + 8, :] for f in range(DH)])
                rd = 1.0 / (dp * rp + dn * rn + 1e-6)
                sp = rp * rd
                sn_ = rn * rd
                ph = jnp.concatenate([t * sp for t in ep] + [t * sn_ for t in en], axis=0).astype(BF16)
                os_.append(_nn(_up(kvm[g]), ph).astype(BF16))
            ot = jnp.concatenate(os_, axis=0)
            bt = _nn(_up(wot[...]), ot)
            gg = jnp.concatenate([gs[:, pl.ds(sn, 128)]] * (D // 8), axis=0)
            res = bt + gg * (at[:, pl.ds(sn, 128)] - bt)
            ob[:, pl.ds(sn, 128)] = res.astype(BF16)
        out_copy(it).start()
        return carry

    jax.lax.fori_loop(0, NIT, phase2, 0)
    for i in range(NIT):
        out_copy(i).wait()


@jax.jit
def pallas_gated_mix__ssm_conv_h3__linear_kernel_hedgehog__prompt_kernel(A_q, A_k, A_v, A_shift_k, A_ssm_k, A_ssm_D, B_x, B_wqkv, B_w_phi, B_wo, gate_w):
    fm, gm = _dft_consts()
    vm = pltpu.VMEM
    scratch = [
        vm((D, S), BF16), vm((D, S), BF16), vm((D, S), BF16), vm((D, S), BF16),
        vm((D, 3 * D), BF16), vm((D, D), BF16),
        vm((4, D), BF16), vm((D,), BF16), vm((D,), BF16), vm((DH, DH, H), BF16),
        vm((B, 2 * B), BF16), vm((2 * B, B), BF16),
        vm((MR // 2, D), U32), vm((D // 2, D), U32),
        vm((5, D, 128), F32),
        vm((CC * NB, 2 * B), F32), vm((NB, CC, 2 * B), F32),
        vm((CC * NB // 2, 2 * B), U32), vm((CC * NB // 2, B), U32),
        vm((D, S), F32), vm((MR, SC), F32),
        vm((NG * 144, SC), U32), vm((D // 2, SC), U32),
        vm((D, S), F32), vm((8, S), F32),
        vm((NG, GR, 288), F32), vm((NG * 288, 128), F32), vm((NG, GR // 2, 288), U32),
        vm((D, S), BF16),
        pltpu.SemaphoreType.DMA((24,)), pltpu.SemaphoreType.DMA((NIT,)),
    ]
    out_t = pl.pallas_call(
        _kernel,
        out_shape=jax.ShapeDtypeStruct((D, S), BF16),
        in_specs=[pl.BlockSpec(memory_space=pl.ANY)] * 12,
        out_specs=pl.BlockSpec(memory_space=pl.ANY),
        scratch_shapes=scratch,
        compiler_params=pltpu.CompilerParams(vmem_limit_bytes=100 * 1024 * 1024),
    )(A_q[0].T, A_k[0].T, A_v[0].T, A_shift_k.T, A_ssm_k, A_ssm_D, B_wqkv,
      jnp.transpose(B_w_phi, (1, 2, 0)), B_wo, gate_w, jnp.asarray(fm, BF16), jnp.asarray(gm, BF16))
    return out_t.T[None]
```

```python
import functools
import math

import jax
import jax.numpy as jnp
import numpy as np
import jax.experimental.pallas as pl
import jax.experimental.pallas.tpu as pltpu

S = 2048
D = 576
H = 32
DH = 18
NG = 8
GR = 72
B = 128
NB = S // B
NIT = 4
CCS = (64, 160, 176, 176)
COFF = tuple(sum(CCS[:i]) for i in range(NIT))
NINV = CCS[2]
C00 = D - 3 * NINV
SC = S // NIT
NT = SC // 128
KD = 544
MR = 2 * KD + D + 16
KO, VO, QO, GO = 0, KD, KD + D, 2 * KD + D
LOG2E = math.log2(math.e)
F32 = jnp.float32
BF16 = jnp.bfloat16
U32 = jnp.uint32
OCH = (2, 2, 2, 2, 2, 2, 2, 1, 1)
QC = 2
SCOPES = False
TRIM = 6
RID0, RIDS, RLAG = 2, 4, 2
USKIP, CAP_U = 20, 24
CAP_R, CAP_K, CAP_V, CAP_I, CAP_RR = 50, 20, 44, 40, 36


def _dft_consts():
    n = np.arange(B, dtype=np.float64)[:, None]
    k = np.arange(B, dtype=np.float64)[None, :]
    ang = 2.0 * np.pi * (2.0 * k + 0.5) * n / (2 * B)
    f = np.concatenate([np.cos(ang), -np.sin(ang)], axis=1)
    g = f.T / B
    return f.astype(np.float32), g.astype(np.float32)


def _nn(a, b):
    return jnp.dot(a, b, preferred_element_type=F32)


def _nt(a, b):
    return jax.lax.dot_general(a, b, (((1,), (1,)), ((), ())), preferred_element_type=F32)


def _pk(x):
    return pltpu.bitcast(x, U32)


def _up(x):
    return pltpu.bitcast(x, BF16)


def _cat(xs, axis=0):
    return xs[0] if len(xs) == 1 else jnp.concatenate(xs, axis=axis)


def _fold8(op, xs):
    r = functools.reduce(op, xs)
    return op(r, pltpu.roll(r, 4, 0))


def _rcp(x):
    return pl.reciprocal(x, approx=True)


def _groups_of_tile(t, off):
    lo = max(0, (128 * t - off) // GR)
    hi = min(NG - 1, (128 * t + 127 - off) // GR)
    return list(range(lo, hi + 1))


def _ds(start, size, align):
    if not isinstance(start, int):
        start = pl.multiple_of(start, align)
    return pl.ds(start, size)


class _Scope:
    def __init__(self, name):
        self.cm = jax.named_scope(name) if SCOPES else None

    def __enter__(self):
        if self.cm is not None:
            self.cm.__enter__()

    def __exit__(self, *a):
        if self.cm is not None:
            self.cm.__exit__(*a)


def _kernel(x_hbm, k_hbm, v_hbm, sk_hbm, h_hbm, sd_hbm, w_hbm, wp_hbm, wo_hbm, gw_hbm, f_hbm, g_hbm,
            o_hbm,
            xb, kb, vb, hb, wb, wob, skb, sdb, gwb, wpb, fb, gb,
            wt, wot, wot2, cb, aps, emat, at, pq, gs, ob, ys0, ys, pkb0, pkb1, pkb2,
            phm, phl, vgp, vnp, kvam, kval, zl,
            sems):
    bump = [0, pkb0]

    def _pb(x):
        n = x.shape[0] // 2
        r, pkb = bump
        bump[0] += n
        pkb[r:r + n, 0:128] = _pk(x.astype(BF16))
        return pkb[r:r + n, 0:128]

    def get_never():
        return fb[0:16, 0:128].astype(F32)[0:8] > 2.0

    def cp(i, src, dst):
        return pltpu.make_async_copy(src, dst, sems.at[i])

    def step_copies(i, sem):
        rs = pl.ds(COFF[i], CCS[i])
        cs = pl.ds(i * SC, SC)
        return ([cp(sem[0], x_hbm.at[:, cs], xb.at[:, cs])],
                [cp(sem[1], s_.at[rs, :], d_.at[rs, :]) for s_, d_ in ((h_hbm, hb), (k_hbm, kb), (v_hbm, vb))])

    x0_, a0_ = step_copies(0, (3, 4))
    grp = [
        [cp(0, wp_hbm, wpb)],
        [cp(1, w_hbm.at[:, 512:1152], wb.at[:, 512:1152])],
        [cp(2, w_hbm.at[:, 0:512], wb.at[:, 0:512])],
        x0_ + [cp(3, sk_hbm, skb), cp(3, sd_hbm, sdb), cp(3, gw_hbm, gwb)],
        [cp(4, f_hbm, fb), cp(4, w_hbm.at[:, 1152:1728], wb.at[:, 1152:1728])] + a0_,
        sum(step_copies(1, (5, 5)), []) + [cp(5, g_hbm, gb), cp(5, wo_hbm, wob)],
        sum(step_copies(2, (6, 6)), []) + sum(step_copies(3, (6, 6)), []),
    ]
    for g_ in grp:
        for c in g_:
            c.start()

    def wait(i):
        with _Scope('wait%d' % i):
            for c in grp[i]:
                c.wait()

    lane = jax.lax.broadcasted_iota(jnp.int32, (8, 128), 1)
    sub = jax.lax.broadcasted_iota(jnp.int32, (8, 128), 0)

    er = jax.lax.broadcasted_iota(jnp.int32, (D, 640), 0)
    ec = jax.lax.broadcasted_iota(jnp.int32, (D, 640), 1)
    emat[...] = _pk(jnp.where(ec == 64 + DH * (er & 31) + (er >> 5), 1.0, 0.0).astype(BF16))
    wait(0)
    tcat = _cat([wpb[d].astype(F32) for d in range(DH)], axis=1)
    amat = _nn(tcat.astype(BF16), _up(emat[...]))
    sub5 = jax.lax.broadcasted_iota(jnp.int32, (8, 640), 0)
    aps[1] = _cat([jnp.where(sub5 < 4, jnp.broadcast_to(amat[2 * fp:2 * fp + 1], (8, 640)),
                             jnp.broadcast_to(amat[2 * fp + 1:2 * fp + 2], (8, 640))) for fp in range(9)])

    def fold(which, off, t0, ro):
        parts = [None] * NG
        for t in range(5):
            gl = _groups_of_tile(t, off)
            a_t = aps[which, :, 128 * t:128 * (t + 1)]
            lhs = []
            for g in gl:
                lo = DH * (4 * g + (sub & 3)) + off - 128 * t
                msk = jnp.logical_and(lane >= lo, lane < lo + DH)
                lhs += [jnp.where(msk, a_t[fp * 8:fp * 8 + 8], 0.0) for fp in range(9)]
            r = _nt(_cat(lhs).astype(BF16), wb[:, 128 * (t0 + t):128 * (t0 + t + 1)])
            for i, g in enumerate(gl):
                piece = r[i * GR:(i + 1) * GR]
                parts[g] = piece if parts[g] is None else parts[g] + piece
        subd = jax.lax.broadcasted_iota(jnp.int32, (8, D), 0)
        out = []
        for p in range(NG // 2):
            us_, ds_ = [], []
            for g in (2 * p, 2 * p + 1):
                s0 = parts[g][0:8]
                r0 = jnp.where(subd < 4, s0, pltpu.roll(s0, 4, 0))
                us_.append(s0 - r0)
                ds_ += [parts[g][fp * 8:fp * 8 + 8] - r0 for fp in range(1, 9)]
            out += [pltpu.roll(us_[0], 4, 0) + us_[1]] + ds_
        wt[ro // 2:(ro + KD) // 2, :] = _pk((_cat(out) * LOG2E).astype(BF16))

    def logits(get, g):
        base = (g // 2) * 136
        x = get(base)
        if g % 2 == 0:
            x = pltpu.roll(x, 4, 0)
        return [jnp.where(sub < 4, 0.0, x)] + [get(base + 8 + (g % 2) * 64 + f * 8) for f in range(8)]

    def project(r0, r1, s0, toks=None, riders=None):
        xv = xb.at[:, _ds(s0, SC, 128)]
        lhs = wt[r0 // 2:r1 // 2, 512:D]
        if riders:
            never = get_never()[:, 0:64]
            riders = list(riders)
            blks = [lhs[r:r + 8] for r in range(0, (r1 - r0) // 2, 8)]
            for i in range(len(blks) - (len(riders) + 1) // 2, len(blks)):
                for _ in range(2):
                    if riders:
                        blks[i] = jnp.where(never, riders.pop(0)[:, 0:64], blks[i])
            lhs = _cat(blks)
        rr = _nn(_up(lhs), xv[512:D, :])
        if toks is not None:
            for r in range(0, r1 - r0, 16):
                toks.append((rr[r:r + 8, 0:128], CAP_R if riders is None else CAP_RR))

        def tile(n):
            pr = _nn(_up(wt[r0 // 2:r1 // 2, 0:512]), xv[0:512, n * 128:(n + 1) * 128]) + rr[:, n * 128:(n + 1) * 128]
            if toks is not None:
                for r in range(0, r1 - r0, 16):
                    toks.append((pr[r:r + 8], CAP_K if r0 + r < VO else CAP_V))
            return pr
        return tile

    def softmax_k(pk, n):
        lefts = []
        for g in range(NG):
            p = logits(lambda r: pk[r:r + 8], g)
            mx = _fold8(jnp.maximum, p)
            mn = _fold8(jnp.minimum, p)
            ep = [jnp.exp2(t - mx) for t in p]
            en = [jnp.exp2(mn - t) for t in p]
            rp = _rcp(_fold8(jnp.add, ep))
            rn = _rcp(_fold8(jnp.add, en))
            ph = [t * rp for t in ep] + [t * rn for t in en]
            phm[g * 64:(g + 1) * 64, n * 128:(n + 1) * 128] = _pk(_cat(ph[0:16]).astype(BF16))
            lefts += ph[16:18]
        left = _cat(lefts)
        phl[:, n * 128:(n + 1) * 128] = _pk(left.astype(BF16))
        return left

    def add_zl(lefts, first):
        tot = functools.reduce(jnp.add, lefts)
        zl[...] = tot if first else zl[...] + tot

    def pack_v(v, n):
        ones = jnp.ones((8, 128), F32)
        vgp[:, n * 128:(n + 1) * 128] = _pk(_cat(sum([[v[g * GR:(g + 1) * GR], ones] for g in range(NG)], [])).astype(BF16))
        vnp[:, n * 128:(n + 1) * 128] = _pk(v.astype(BF16))

    def kv_state(first):
        res_m, res_l = [], []
        for g in range(NG):
            r = _nt(_up(vgp[g * 40:(g + 1) * 40, :]), _up(phm[g * 64:(g + 1) * 64, :]))
            res_m.append(r if first else kvam[g] + r)
            kvam[g] = res_m[-1]
        for t in range(5):
            gl = _groups_of_tile(t, 0)
            hi = min(D, 128 * (t + 1))
            r = _nt(_up(phl[gl[0] * 8:(gl[-1] + 1) * 8, :]), _up(vnp[64 * t:hi // 2, :]))
            res_l.append(r if first else kval[0:16 * len(gl), 128 * t:hi] + r)
            kval[0:16 * len(gl), 128 * t:hi] = res_l[-1]
        return res_m, res_l

    def store_q(pr, off, sn):
        pq[:, _ds(sn, 128, 128)] = pr[off:off + KD]
        gs[:, _ds(sn, 128, 128)] = jax.nn.sigmoid(pr[off + KD:off + KD + 8])

    def filter_spec(c0, nc):
        hv = hb.at[_ds(c0, nc, 16), :]
        dv = cb.at[4, _ds(c0, nc, 16), :]
        hl = _cat([hv[16 * cg:16 * cg + 16, m * B:(m + 1) * B] for cg in range(nc // 16) for m in range(NB)])
        hr = _nn(hl, fb[...])

        def spec(rg, m):
            r = (rg // 2) * 256 + m * 16 + (rg % 2) * 8
            cur = hr[r:r + 8]
            if m == 0:
                return cur[:, 0:B] + dv[rg * 8:rg * 8 + 8, :], cur[:, B:2 * B]
            prv = hr[r - 16:r - 8]
            return cur[:, 0:B] - prv[:, B:2 * B], cur[:, B:2 * B] + prv[:, 0:B]
        return [[spec(rg, m) for m in range(NB)] for rg in range(nc // 8)]

    def data_spec(c0, nc, toks):
        kv_ = kb.at[_ds(c0, nc, 16), :]
        vv_ = vb.at[_ds(c0, nc, 16), :]
        cv = cb.at[:, _ds(c0, nc, 16), :]
        kvs = []
        for rg in range(nc // 8):
            r = rg * 8
            co = [cv[t, r:r + 8, :] for t in range(4)]
            kf = kv_[r:r + 8, :].astype(F32)
            vf = vv_[r:r + 8, :].astype(F32)
            p1 = jnp.zeros((8, 128), F32)
            p2 = jnp.zeros((8, 128), F32)
            outs = []
            for j in range(NB):
                kj = kf[:, j * B:(j + 1) * B]
                r1 = pltpu.roll(kj, 1, 1)
                k1 = jnp.where(lane < 1, p1, r1)
                p1 = r1
                a = co[0] * kj + co[1] * k1
                b = co[2] * kj + co[3] * k1
                r2 = pltpu.roll(b, 2, 1)
                b2 = jnp.where(lane < 2, p2, r2)
                p2 = r2
                outs.append((a + b2) * vf[:, j * B:(j + 1) * B])
            kvs.append(_pb(_cat(outs)))
        ur = _nn(_up(_cat(kvs)), fb[...])
        for r in range(USKIP * 16, nc * NB, 16):
            toks.append((ur[r:r + 8, 0:B], CAP_U))
        return ur

    def mac_all(hs, ur, dest, nc, toks):
        never = get_never()
        nrg = nc // 8
        total = nrg * (136 * 8 + 80)
        cap = sum(c for _, c in toks)
        scale = total / cap
        st = {'i': 0, 'room': toks[0][1] * scale}

        def token(cost):
            while st['room'] < cost * 0.5 and st['i'] + 1 < len(toks):
                st['i'] += 1
                st['room'] += toks[st['i']][1] * scale
            st['room'] -= cost
            return toks[st['i']][0]

        for rg in range(nrg):
            for i0 in range(0, NB, 4):
                acc = [None] * 4
                for j in range(i0 + 4):
                    u_re = ur[rg * 128 + j * 8:rg * 128 + j * 8 + 8, 0:B]
                    u_im = ur[rg * 128 + j * 8:rg * 128 + j * 8 + 8, B:2 * B]
                    na = min(4, i0 + 4 - j)
                    tk_ = token(8 * na + 2)
                    u_re = jnp.where(never, tk_, u_re)
                    u_im = jnp.where(never, tk_, u_im)
                    for a in range(4):
                        m = i0 + a - j
                        if m < 0:
                            continue
                        h_re, h_im = hs[rg][m]
                        t_re = h_re * u_re - h_im * u_im
                        t_im = h_re * u_im + h_im * u_re
                        acc[a] = (t_re, t_im) if acc[a] is None else (acc[a][0] + t_re, acc[a][1] + t_im)
                yv, slot = dest(rg)
                r0 = slot * 64 + i0 * 4
                yv[r0:r0 + 16, 0:B] = _pk(_cat([t[0] for t in acc]).astype(BF16))
                yv[r0:r0 + 16, B:2 * B] = _pk(_cat([t[1] for t in acc]).astype(BF16))

    def conv_out(yv, c0, nc, toks=None):
        hf = nc * 4
        av = at.at[_ds(c0, nc, 16), :]
        yr = _cat([_nn(_up(yv[0:hf]), gb[...]), _nn(_up(yv[hf:2 * hf]), gb[...])])
        if toks is not None:
            for r in range(0, 2 * hf, 16):
                toks.append((yr[r:r + 8], CAP_I))
        for rg in range(nc // 8):
            for i in range(NB):
                av[rg * 8:rg * 8 + 8, i * B:(i + 1) * B] = yr[rg * 128 + i * 8:rg * 128 + i * 8 + 8]

    wait(1)
    fold(1, 64, 4, KO)
    aps[0] = pltpu.roll(aps[1], 640 - 64, 1)
    wait(2)
    fold(0, 0, 0, QO)

    wait(3)
    skf = skb[...].astype(F32)
    for t in range(4):
        cb[t] = jnp.broadcast_to(skf[t:t + 1, :], (128, D)).T
    cb[4] = jnp.broadcast_to(sdb[...].astype(F32).reshape(1, D), (128, D)).T
    wt[GO // 2:GO // 2 + 8, :] = _pk(jnp.broadcast_to(gwb[...].astype(F32).reshape(1, D), (16, D)).astype(BF16))
    tk = project(KO, KO + KD, 0)
    add_zl([softmax_k(tk(n), n) for n in range(NT)], True)
    toks = []
    tq = project(QO, MR, 0, toks)
    for n in range(QC):
        store_q(tq(n), 0, n * 128)

    wait(4)
    wt[VO // 2:(VO + D) // 2, :] = _pk(wb[:, 2 * D:3 * D].astype(F32).T.astype(BF16))
    store_q(tq(QC), 0, QC * 128)
    del toks[:]
    hs = filter_spec(0, CCS[0])
    ur = data_spec(0, CCS[0], toks)
    for n in range(QC + 1, NT):
        store_q(tq(n), 0, n * 128)
    tv = project(VO, VO + D, 0, toks)
    for n in range(NT):
        pack_v(tv(n), n)
    mac_all(hs, ur, lambda rg: (ys0, rg) if rg < C00 // 8 else (ys, rg - C00 // 8), CCS[0], toks[:-TRIM])

    def step(c0, nc, s0, ic0, inc, first):
        toks = []
        kv_state(first)
        hs = filter_spec(c0, nc)
        ur = data_spec(c0, nc, toks)
        riders = None
        if first:
            wot[...] = _pk(wob[...].astype(F32).T.astype(BF16))
            wot2[...] = jnp.zeros(wot2.shape, U32)
            wot2[:, 0:64] = wot[:, 512:D]
            riders = []
            for q in range(0, D // 2, 8):
                riders += [wot[q:q + 8, 128 * t:128 * (t + 1)] for t in range(4)] + [wot2[q:q + 8, :]]
        conv_out(ys0 if first else ys, ic0, inc, toks)
        tl = project(0, MR, s0, toks, riders)
        lefts = []
        for n in range(NT):
            pr = tl(n)
            lefts.append(softmax_k(pr, n))
            pack_v(pr[VO:VO + D], n)
            store_q(pr, QO, s0 + n * 128)
        add_zl(lefts, False)
        mac_all(hs, ur, lambda rg: (ys, rg + (NINV - nc) // 8), nc, toks[:-TRIM])

    wait(5)
    step(COFF[1], CCS[1], SC, 0, C00, True)
    wait(6)

    def loop_body(i, carry):
        bump[:] = [0, pkb1]
        step(COFF[2] + i * CCS[2], CCS[2], (2 + i) * SC, C00 + i * NINV, NINV, False)
        return carry

    with _Scope('loop'):
        jax.lax.fori_loop(0, 2, loop_body, 0)

    bump[:] = [0, pkb2]
    never = get_never()
    toks0 = []
    acc_m, acc_l = kv_state(False)
    conv_out(ys, D - NINV, NINV, toks0)
    rh = jax.lax.broadcasted_iota(jnp.int32, (80, 128), 0)
    ch = jax.lax.broadcasted_iota(jnp.int32, (80, 128), 1) & 3
    kmask = jnp.logical_and(rh >= DH * ch, rh < DH * ch + DH)
    kvm = [jnp.where(kmask, acc_m[g], 0.0).astype(BF16) for g in range(NG)]
    zm = [_cat([acc_m[g][GR:GR + 8, :]] * 16).T for g in range(NG)]
    zlb = jnp.broadcast_to(jnp.sum(zl[...], axis=1, keepdims=True), (128, 128))
    kl_t = []
    for t in range(5):
        gl = _groups_of_tile(t, 0)
        wd = min(D, 128 * (t + 1)) - 128 * t
        rl = jax.lax.broadcasted_iota(jnp.int32, (16 * len(gl), wd), 0) + 16 * gl[0]
        cl = jax.lax.broadcasted_iota(jnp.int32, (16 * len(gl), wd), 1) + 128 * t
        hl_ = 4 * (rl >> 4) + (rl & 3)
        blk = jnp.where(jnp.logical_and(cl >= DH * hl_, cl < DH * hl_ + DH), acc_l[t], 0.0)
        parts = []
        if gl[0] > 0:
            parts.append(jnp.zeros((16 * gl[0], wd), F32))
        parts.append(blk)
        if gl[-1] < NG - 1:
            parts.append(jnp.zeros((16 * (NG - 1 - gl[-1]), wd), F32))
        kl_t.append(_pb(_cat(parts).T))
    kvl = _cat(kl_t)
    wfl = _nn(_up(wot[:, 256:D]), _up(kvl[128:D // 2]))
    lane_b = jax.lax.broadcasted_iota(jnp.int32, (D // 2, 128), 1)
    wrem = jnp.where(lane_b < 64, wot2[...], _pb(wfl))

    ostart = [sum(OCH[:i]) for i in range(len(OCH))]

    def out_copy(i):
        sl = pl.ds(ostart[i] * 128, OCH[i] * 128)
        return cp(7, ob.at[:, sl], o_hbm.at[:, sl])

    def attn_phi(n, toks):
        mains, lefts, done = [], [], []
        for g in range(NG):
            p = logits(lambda r: pq[r:r + 8, n * 128:(n + 1) * 128], g)
            if toks is not None:
                p[1] = jnp.where(never, toks[g], p[1])
            mx = _fold8(jnp.maximum, p)
            mn = _fold8(jnp.minimum, p)
            e = [jnp.exp2(t - mx) for t in p] + [jnp.exp2(mn - t) for t in p]
            rp = _rcp(_fold8(jnp.add, e[0:9]))
            rn = _rcp(_fold8(jnp.add, e[9:18]))
            z = [zm[g][i * 8:(i + 1) * 8] for i in range(16)] + [zlb[g * 16 + i * 8:g * 16 + i * 8 + 8] for i in range(2)]
            dp = functools.reduce(jnp.add, [e[i] * z[i] for i in range(9)])
            dn = functools.reduce(jnp.add, [e[i] * z[i] for i in range(9, 18)])
            dh = dp * rp + dn * rn
            rd = _rcp(dh + pltpu.roll(dh, 4, 0) + 1e-6)
            sp = rp * rd
            sn_ = rn * rd
            ph = [t * sp for t in e[0:9]] + [t * sn_ for t in e[9:18]]
            mains.append(_cat(ph[0:16]).astype(BF16))
            lefts += ph[16:18]
            done.append(pltpu.bitcast(sn_, U32))
        return mains, _pb(_cat(lefts)), done

    def attn_o(phi):
        mains, left, _ = phi
        om = _cat([_nn(kvm[g], mains[g])[0:GR] for g in range(NG)])
        ol = _cat([_nn(_up(kvl[72 * q:72 * (q + 1), 0:64]), _up(left[0:32])) for q in range(2)])
        return om, _cat([_pb(_cat([om[0:288] + ol, om[288:D]])), left[32:64]])

    def finish(n, ot, riders=None):
        br = _cat([_nn(_up(wrem[72 * q:72 * (q + 1)]), _up(ot[256:320])) for q in range(4)])
        w0 = wot[:, 0:128]
        if riders:
            blks = [w0[r:r + 8] for r in range(0, D // 2, 8)]
            for g in range(NG):
                blks[RID0 + RIDS * g] = jnp.where(never, riders[g], blks[RID0 + RIDS * g])
            w0 = _cat(blks)
        bt = _nn(_up(_cat([w0, wot[:, 128:512]], axis=1)), _up(ot[0:256])) + br
        gg = _cat([gs[:, n * 128:(n + 1) * 128]] * (D // 8))
        a = at[:, n * 128:(n + 1) * 128] * xb[:, n * 128:(n + 1) * 128].astype(F32)
        ob[:, n * 128:(n + 1) * 128] = (bt + gg * (a - bt)).astype(BF16)
        for i in range(len(OCH)):
            if n + 1 == ostart[i] + OCH[i]:
                out_copy(i).start()
        return br, bt

    nt0 = len(toks0)
    phi = {0: attn_phi(0, None),
           1: attn_phi(1, [toks0[(nt0 * g) // 16][0] for g in range(NG)]),
           2: attn_phi(2, [toks0[(nt0 * (g + 8)) // 16][0] for g in range(NG)])}
    om0, o0 = attn_o(phi[0])
    om1, o1 = attn_o(phi[1])
    ot = {0: o0, 1: o1}
    phi[3] = attn_phi(3, [om0[GR * g:GR * g + 8] for g in range(0, 8, 2)] + [om1[GR * g:GR * g + 8] for g in range(0, 8, 2)])
    for n in range(NB):
        br, bt = finish(n, ot[n], phi[n + RLAG][2] if n + RLAG < NB else None)
        if n + 2 < NB:
            om, ot[n + 2] = attn_o(phi[n + 2])
        if n + 4 < NB:
            tk = [br[0:8], bt[64:72], bt[208:216], bt[352:360], bt[496:504], om[0:8], om[4 * GR:4 * GR + 8], om[7 * GR + 64:7 * GR + 72]]
            phi[n + 4] = attn_phi(n + 4, tk)
    with _Scope('wait_out'):
        for i in range(len(OCH)):
            out_copy(i).wait()


@jax.jit
def pallas_gated_mix__ssm_conv_h3__linear_kernel_hedgehog__prompt_kernel(A_q, A_k, A_v, A_shift_k, A_ssm_k, A_ssm_D, B_x, B_wqkv, B_w_phi, B_wo, gate_w):
    fm, gm = _dft_consts()
    vm = pltpu.VMEM
    scratch = [
        vm((D, S), BF16), vm((D, S), BF16), vm((D, S), BF16), vm((D, S), BF16),
        vm((D, 3 * D), BF16), vm((D, D), BF16),
        vm((4, D), BF16), vm((D,), BF16), vm((D,), BF16), vm((DH, DH, H), BF16),
        vm((B, 2 * B), BF16), vm((2 * B, B), BF16),
        vm((MR // 2, D), U32), vm((D // 2, D), U32), vm((D // 2, 128), U32),
        vm((5, D, 128), F32), vm((2, GR, 640), F32), vm((D // 2, 640), U32),
        vm((D, S), F32), vm((KD, S), F32), vm((8, S), F32),
        vm((D, S), BF16), vm((C00 * 8, 2 * B), U32), vm((NINV * 8, 2 * B), U32),
        vm((8 * (CCS[0] + CCS[1]), 256), U32), vm((8 * CCS[2], 256), U32), vm((D + NB * 352, 256), U32),
        vm((NG * 64, SC), U32), vm((NG * 8, SC), U32),
        vm((NG * 40, SC), U32), vm((D // 2, SC), U32),
        vm((NG, 80, 128), F32), vm((48, D), F32), vm((128, 128), F32),
        pltpu.SemaphoreType.DMA((8,)),
    ]
    out_t = pl.pallas_call(
        _kernel,
        out_shape=jax.ShapeDtypeStruct((D, S), BF16),
        in_specs=[pl.BlockSpec(memory_space=pl.ANY)] * 12,
        out_specs=pl.BlockSpec(memory_space=pl.ANY),
        scratch_shapes=scratch,
        compiler_params=pltpu.CompilerParams(vmem_limit_bytes=100 * 1024 * 1024),
    )(A_q[0].T, A_k[0].T, A_v[0].T, A_shift_k.T, A_ssm_k, A_ssm_D, B_wqkv,
      jnp.transpose(B_w_phi, (1, 2, 0)), B_wo, gate_w, jnp.asarray(fm, BF16), jnp.asarray(gm, BF16))
    return out_t.T[None]
```

```python
import functools
import math

import jax
import jax.numpy as jnp
import numpy as np
import jax.experimental.pallas as pl
import jax.experimental.pallas.tpu as pltpu

S = 2048
D = 576
H = 32
DH = 18
NG = 8
GR = 72
B = 128
NB = S // B
NIT = 4
CCS = (64, 160, 176, 176)
COFF = tuple(sum(CCS[:i]) for i in range(NIT))
NINV = CCS[2]
C00 = D - 3 * NINV
SC = S // NIT
NT = SC // 128
KD = 544
MR = 2 * KD + D + 16
KO, VO, GO, QO = 0, KD, KD + D, KD + D + 16
LOG2E = math.log2(math.e)
F32 = jnp.float32
BF16 = jnp.bfloat16
U32 = jnp.uint32
OCH = (2, 2, 2, 2, 2, 2, 2, 1, 1)
QC = 2
SCOPES = False
TRIM = 6
LAST = (0, 384, 512, 576)
RID0, RIDS, RLAG = 2, 4, 2
USKIP, CAP_U = 20, 24
CAP_R, CAP_K, CAP_V, CAP_I, CAP_RR = 50, 20, 44, 40, 36


def _dft_consts():
    n = np.arange(B, dtype=np.float64)[:, None]
    k = np.arange(B, dtype=np.float64)[None, :]
    ang = 2.0 * np.pi * (2.0 * k + 0.5) * n / (2 * B)
    f = np.concatenate([np.cos(ang), -np.sin(ang)], axis=1)
    g = f.T / B
    return f.astype(np.float32), g.astype(np.float32)


def _nn(a, b):
    return jnp.dot(a, b, preferred_element_type=F32)


def _nt(a, b):
    return jax.lax.dot_general(a, b, (((1,), (1,)), ((), ())), preferred_element_type=F32)


def _pk(x):
    return pltpu.bitcast(x, U32)


def _up(x):
    return pltpu.bitcast(x, BF16)


def _cat(xs, axis=0):
    return xs[0] if len(xs) == 1 else jnp.concatenate(xs, axis=axis)


def _fold8(op, xs):
    r = functools.reduce(op, xs)
    return op(r, pltpu.roll(r, 4, 0))


def _rcp(x):
    return pl.reciprocal(x, approx=True)


def _groups_of_tile(t, off):
    lo = max(0, (128 * t - off) // GR)
    hi = min(NG - 1, (128 * t + 127 - off) // GR)
    return list(range(lo, hi + 1))


def _ds(start, size, align):
    if not isinstance(start, int):
        start = pl.multiple_of(start, align)
    return pl.ds(start, size)


class _Scope:
    def __init__(self, name):
        self.cm = jax.named_scope(name) if SCOPES else None

    def __enter__(self):
        if self.cm is not None:
            self.cm.__enter__()

    def __exit__(self, *a):
        if self.cm is not None:
            self.cm.__exit__(*a)


def _kernel(x_hbm, k_hbm, v_hbm, sk_hbm, h_hbm, sd_hbm, w_hbm, wp_hbm, wo_hbm, gw_hbm, f_hbm, g_hbm,
            o_hbm,
            xb, kb, vb, hb, wb, wob, skb, sdb, gwb, wpb, fb, gb,
            wt, wot, wot2, cb, aps, emat, at, pq, gs, ob, ys0, ys, pkb0, pkb1, pkb2,
            phm, phl, vgp, vnp, kvam, kval, zl,
            sems):
    bump = [0, pkb0]

    def _pb(x):
        n = x.shape[0] // 2
        r, pkb = bump
        bump[0] += n
        pkb[r:r + n, 0:128] = _pk(x.astype(BF16))
        return pkb[r:r + n, 0:128]

    def get_never():
        return fb[0:16, 0:128].astype(F32)[0:8] > 2.0

    def cp(i, src, dst):
        return pltpu.make_async_copy(src, dst, sems.at[i])

    def step_copies(i, sem):
        rs = pl.ds(COFF[i], CCS[i])
        cs = pl.ds(i * SC, SC)
        return ([cp(sem[0], x_hbm.at[:, cs], xb.at[:, cs])],
                [cp(sem[1], s_.at[rs, :], d_.at[rs, :]) for s_, d_ in ((h_hbm, hb), (k_hbm, kb), (v_hbm, vb))])

    x0_, a0_ = step_copies(0, (3, 4))
    grp = [
        [cp(0, wp_hbm, wpb)],
        [cp(1, w_hbm.at[:, 768:1152], wb.at[:, 768:1152])],
        [cp(2, w_hbm.at[:, 384:768], wb.at[:, 384:768])],
        x0_ + [cp(3, sk_hbm, skb), cp(3, sd_hbm, sdb), cp(3, gw_hbm, gwb)],
        [cp(4, f_hbm, fb), cp(4, w_hbm.at[:, 1152:1728], wb.at[:, 1152:1728])] + a0_,
        sum(step_copies(1, (5, 5)), []) + [cp(5, g_hbm, gb), cp(5, wo_hbm, wob)],
        sum(step_copies(2, (6, 6)), []) + sum(step_copies(3, (6, 6)), []),
        [cp(8, w_hbm.at[:, 0:384], wb.at[:, 0:384])],
    ]
    for c in grp[0] + grp[1] + grp[3][1:] + grp[2] + grp[7] + grp[3][:1] + grp[4] + grp[5] + grp[6]:
        c.start()

    def wait(i):
        with _Scope('wait%d' % i):
            for c in grp[i]:
                c.wait()

    lane = jax.lax.broadcasted_iota(jnp.int32, (8, 128), 1)
    sub = jax.lax.broadcasted_iota(jnp.int32, (8, 128), 0)

    er = jax.lax.broadcasted_iota(jnp.int32, (D, 640), 0)
    ec = jax.lax.broadcasted_iota(jnp.int32, (D, 640), 1)
    emat[...] = _pk(jnp.where(ec == 64 + DH * (er & 31) + (er >> 5), 1.0, 0.0).astype(BF16))
    wait(0)
    tcat = _cat([wpb[d].astype(F32) for d in range(DH)], axis=1)
    amat = _nn(tcat.astype(BF16), _up(emat[...]))
    sub5 = jax.lax.broadcasted_iota(jnp.int32, (8, 640), 0)
    aps[1] = _cat([jnp.where(sub5 < 4, jnp.broadcast_to(amat[2 * fp:2 * fp + 1], (8, 640)),
                             jnp.broadcast_to(amat[2 * fp + 1:2 * fp + 2], (8, 640))) for fp in range(9)])

    def fold_mm(parts, which, off, t0, tiles):
        for t in tiles:
            gl = _groups_of_tile(t, off)
            a_t = aps[which, :, 128 * t:128 * (t + 1)]
            lhs = []
            for g in gl:
                lo = DH * (4 * g + (sub & 3)) + off - 128 * t
                msk = jnp.logical_and(lane >= lo, lane < lo + DH)
                lhs += [jnp.where(msk, a_t[fp * 8:fp * 8 + 8], 0.0) for fp in range(9)]
            r = _nt(_cat(lhs).astype(BF16), wb[:, 128 * (t0 + t):128 * (t0 + t + 1)])
            for i, g in enumerate(gl):
                piece = r[i * GR:(i + 1) * GR]
                parts[g] = piece if parts[g] is None else parts[g] + piece

    def fold_out(parts, ro, pairs):
        subd = jax.lax.broadcasted_iota(jnp.int32, (8, D), 0)
        out = []
        for p in pairs:
            us_, ds_ = [], []
            for g in (2 * p, 2 * p + 1):
                s0 = parts[g][0:8]
                r0 = jnp.where(subd < 4, s0, pltpu.roll(s0, 4, 0))
                us_.append(s0 - r0)
                ds_ += [parts[g][fp * 8:fp * 8 + 8] - r0 for fp in range(1, 9)]
            out += [pltpu.roll(us_[0], 4, 0) + us_[1]] + ds_
        r0 = (ro + 136 * pairs[0]) // 2
        wt[r0:r0 + 68 * len(pairs), :] = _pk((_cat(out) * LOG2E).astype(BF16))

    def logits(get, g):
        base = (g // 2) * 136
        x = get(base)
        if g % 2 == 0:
            x = pltpu.roll(x, 4, 0)
        return [jnp.where(sub < 4, 0.0, x)] + [get(base + 8 + (g % 2) * 64 + f * 8) for f in range(8)]

    def project(r0, r1, s0, toks=None, riders=None):
        xv = xb.at[:, _ds(s0, SC, 128)]
        lhs = wt[r0 // 2:r1 // 2, 512:D]
        if riders:
            never = get_never()[:, 0:64]
            riders = list(riders)
            blks = [lhs[r:r + 8] for r in range(0, (r1 - r0) // 2, 8)]
            for i in range(len(blks) - (len(riders) + 1) // 2, len(blks)):
                for _ in range(2):
                    if riders:
                        blks[i] = jnp.where(never, riders.pop(0)[:, 0:64], blks[i])
            lhs = _cat(blks)
        rr = _nn(_up(lhs), xv[512:D, :])
        if toks is not None:
            for r in range(0, r1 - r0, 16):
                toks.append((rr[r:r + 8, 0:128], CAP_R if riders is None else CAP_RR))

        def tile(n):
            pr = _nn(_up(wt[r0 // 2:r1 // 2, 0:512]), xv[0:512, n * 128:(n + 1) * 128]) + rr[:, n * 128:(n + 1) * 128]
            if toks is not None:
                for r in range(0, r1 - r0, 16):
                    toks.append((pr[r:r + 8], CAP_K if r0 + r < VO else CAP_V))
            return pr
        return tile

    def softmax_k(pk, n):
        lefts = []
        for g in range(NG):
            p = logits(lambda r: pk[r:r + 8], g)
            mx = _fold8(jnp.maximum, p)
            mn = _fold8(jnp.minimum, p)
            ep = [jnp.exp2(t - mx) for t in p]
            en = [jnp.exp2(mn - t) for t in p]
            rp = _rcp(_fold8(jnp.add, ep))
            rn = _rcp(_fold8(jnp.add, en))
            ph = [t * rp for t in ep] + [t * rn for t in en]
            phm[g * 64:(g + 1) * 64, n * 128:(n + 1) * 128] = _pk(_cat(ph[0:16]).astype(BF16))
            lefts += ph[16:18]
        left = _cat(lefts)
        phl[:, n * 128:(n + 1) * 128] = _pk(left.astype(BF16))
        return left

    def add_zl(lefts, first):
        tot = functools.reduce(jnp.add, lefts)
        zl[...] = tot if first else zl[...] + tot

    def pack_v(v, n):
        ones = jnp.ones((8, 128), F32)
        vgp[:, n * 128:(n + 1) * 128] = _pk(_cat(sum([[v[g * GR:(g + 1) * GR], ones] for g in range(NG)], [])).astype(BF16))
        vnp[:, n * 128:(n + 1) * 128] = _pk(v.astype(BF16))

    def kv_state(first):
        res_m, res_l = [], []
        for g in range(NG):
            r = _nt(_up(vgp[g * 40:(g + 1) * 40, :]), _up(phm[g * 64:(g + 1) * 64, :]))
            res_m.append(r if first else kvam[g] + r)
            kvam[g] = res_m[-1]
        for t in range(5):
            gl = _groups_of_tile(t, 0)
            hi = min(D, 128 * (t + 1))
            r = _nt(_up(phl[gl[0] * 8:(gl[-1] + 1) * 8, :]), _up(vnp[64 * t:hi // 2, :]))
            res_l.append(r if first else kval[0:16 * len(gl), 128 * t:hi] + r)
            kval[0:16 * len(gl), 128 * t:hi] = res_l[-1]
        return res_m, res_l

    def store_q(pr, off, sn):
        gs[:, _ds(sn, 128, 128)] = jax.nn.sigmoid(pr[off:off + 8])
        pq[:, _ds(sn, 128, 128)] = pr[off + 16:off + 16 + KD]

    def filter_spec(c0, nc):
        hv = hb.at[_ds(c0, nc, 16), :]
        dv = cb.at[4, _ds(c0, nc, 16), :]
        hl = _cat([hv[16 * cg:16 * cg + 16, m * B:(m + 1) * B] for cg in range(nc // 16) for m in range(NB)])
        hr = _nn(hl, fb[...])

        def spec(rg, m):
            r = (rg // 2) * 256 + m * 16 + (rg % 2) * 8
            cur = hr[r:r + 8]
            if m == 0:
                return cur[:, 0:B] + dv[rg * 8:rg * 8 + 8, :], cur[:, B:2 * B]
            return cur[:, 0:B], cur[:, B:2 * B]
        return [[spec(rg, m) for m in range(NB)] for rg in range(nc // 8)]

    def data_spec(c0, nc, toks):
        kv_ = kb.at[_ds(c0, nc, 16), :]
        vv_ = vb.at[_ds(c0, nc, 16), :]
        cv = cb.at[:, _ds(c0, nc, 16), :]
        kvs = []
        for rg in range(nc // 8):
            r = rg * 8
            co = [cv[t, r:r + 8, :] for t in range(4)]
            kf = kv_[r:r + 8, :].astype(F32)
            vf = vv_[r:r + 8, :].astype(F32)
            p1 = jnp.zeros((8, 128), F32)
            p2 = jnp.zeros((8, 128), F32)
            outs = []
            for j in range(NB):
                kj = kf[:, j * B:(j + 1) * B]
                r1 = pltpu.roll(kj, 1, 1)
                k1 = jnp.where(lane < 1, p1, r1)
                p1 = r1
                a = co[0] * kj + co[1] * k1
                b = co[2] * kj + co[3] * k1
                r2 = pltpu.roll(b, 2, 1)
                b2 = jnp.where(lane < 2, p2, r2)
                p2 = r2
                outs.append((a + b2) * vf[:, j * B:(j + 1) * B])
            kvs.append(_pb(_cat(outs)))
        ur = _nn(_up(_cat(kvs)), fb[...])
        for r in range(USKIP * 16, nc * NB, 16):
            toks.append((ur[r:r + 8, 0:B], CAP_U))
        return ur

    def mac_all(hs, ur, dest, nc, toks):
        never = get_never()
        nrg = nc // 8
        total = nrg * (136 * 8 + 80)
        cap = sum(c for _, c in toks)
        scale = total / cap
        st = {'i': 0, 'room': toks[0][1] * scale}

        def token(cost):
            while st['room'] < cost * 0.5 and st['i'] + 1 < len(toks):
                st['i'] += 1
                st['room'] += toks[st['i']][1] * scale
            st['room'] -= cost
            return toks[st['i']][0]

        for rg in range(nrg):
            prev = None
            for i0 in range(0, NB, 4):
                acc = [None] * 4
                for j in range(i0 + 4):
                    u_re = ur[rg * 128 + j * 8:rg * 128 + j * 8 + 8, 0:B]
                    u_im = ur[rg * 128 + j * 8:rg * 128 + j * 8 + 8, B:2 * B]
                    na = min(4, i0 + 4 - j)
                    tk_ = token(8 * na + 2)
                    u_re = jnp.where(never, tk_, u_re)
                    u_im = jnp.where(never, tk_, u_im)
                    for a in range(4):
                        m = i0 + a - j
                        if m < 0:
                            continue
                        h_re, h_im = hs[rg][m]
                        t_re = h_re * u_re - h_im * u_im
                        t_im = h_re * u_im + h_im * u_re
                        acc[a] = (t_re, t_im) if acc[a] is None else (acc[a][0] + t_re, acc[a][1] + t_im)
                out = []
                for a in range(4):
                    out.append(acc[a] if prev is None else (acc[a][0] - prev[1], acc[a][1] + prev[0]))
                    prev = acc[a]
                yv, slot = dest(rg)
                r0 = slot * 64 + i0 * 4
                yv[r0:r0 + 16, 0:B] = _pk(_cat([t[0] for t in out]).astype(BF16))
                yv[r0:r0 + 16, B:2 * B] = _pk(_cat([t[1] for t in out]).astype(BF16))

    def conv_out(yv, c0, nc, toks=None):
        hf = nc * 4
        av = at.at[_ds(c0, nc, 16), :]
        yr = _cat([_nn(_up(yv[0:hf]), gb[...]), _nn(_up(yv[hf:2 * hf]), gb[...])])
        if toks is not None:
            for r in range(0, 2 * hf, 16):
                toks.append((yr[r:r + 8], CAP_I))
        for rg in range(nc // 8):
            for i in range(NB):
                av[rg * 8:rg * 8 + 8, i * B:(i + 1) * B] = yr[rg * 128 + i * 8:rg * 128 + i * 8 + 8]

    pk_, pq_ = [None] * NG, [None] * NG
    wait(1)
    fold_mm(pk_, 1, 64, 4, (4, 3, 2))
    fold_out(pk_, KO, (2, 3))
    aps[0] = pltpu.roll(aps[1], 640 - 64, 1)
    wait(2)
    fold_mm(pk_, 1, 64, 4, (1, 0))
    fold_out(pk_, KO, (0, 1))
    fold_mm(pq_, 0, 0, 0, (4, 3))
    wait(7)
    fold_mm(pq_, 0, 0, 0, (2, 1, 0))
    fold_out(pq_, QO, (0, 1, 2, 3))

    wait(3)
    skf = skb[...].astype(F32)
    for t in range(4):
        cb[t] = jnp.broadcast_to(skf[t:t + 1, :], (128, D)).T
    cb[4] = jnp.broadcast_to(sdb[...].astype(F32).reshape(1, D), (128, D)).T
    wt[GO // 2:GO // 2 + 8, :] = _pk(jnp.broadcast_to(gwb[...].astype(F32).reshape(1, D), (16, D)).astype(BF16))
    tk = project(KO, KO + KD, 0)
    add_zl([softmax_k(tk(n), n) for n in range(NT)], True)
    toks = []
    tq = project(GO, MR, 0, toks)
    for n in range(QC):
        store_q(tq(n), 0, n * 128)

    wait(4)
    wt[VO // 2:(VO + D) // 2, :] = _pk(wb[:, 2 * D:3 * D].astype(F32).T.astype(BF16))
    store_q(tq(QC), 0, QC * 128)
    del toks[:]
    hs = filter_spec(0, CCS[0])
    ur = data_spec(0, CCS[0], toks)
    for n in range(QC + 1, NT):
        store_q(tq(n), 0, n * 128)
    tv = project(VO, VO + D, 0, toks)
    for n in range(NT):
        pack_v(tv(n), n)
    mac_all(hs, ur, lambda rg: (ys0, rg) if rg < C00 // 8 else (ys, rg - C00 // 8), CCS[0], toks[:-TRIM])

    def step(c0, nc, s0, ic0, inc, first):
        toks = []
        kv_state(first)
        hs = filter_spec(c0, nc)
        ur = data_spec(c0, nc, toks)
        riders = None
        if first:
            wot[...] = _pk(wob[...].astype(F32).T.astype(BF16))
            wot2[...] = jnp.zeros(wot2.shape, U32)
            wot2[:, 0:64] = wot[:, 512:D]
            riders = []
            for q in range(0, D // 2, 8):
                riders += [wot[q:q + 8, 128 * t:128 * (t + 1)] for t in range(4)] + [wot2[q:q + 8, :]]
        conv_out(ys0 if first else ys, ic0, inc, toks)
        tl = project(0, MR, s0, toks, riders)
        lefts = []
        for n in range(NT):
            pr = tl(n)
            lefts.append(softmax_k(pr, n))
            pack_v(pr[VO:VO + D], n)
            store_q(pr, GO, s0 + n * 128)
        add_zl(lefts, False)
        mac_all(hs, ur, lambda rg: (ys, rg + (NINV - nc) // 8), nc, toks[:-TRIM])

    wait(5)
    step(COFF[1], CCS[1], SC, 0, C00, True)
    wait(6)

    def loop_body(i, carry):
        bump[:] = [0, pkb1]
        step(COFF[2] + i * CCS[2], CCS[2], (2 + i) * SC, C00 + i * NINV, NINV, False)
        return carry

    with _Scope('loop'):
        jax.lax.fori_loop(0, 2, loop_body, 0)

    bump[:] = [0, pkb2]
    never = get_never()
    toks0 = []
    acc_m, acc_l = kv_state(False)
    conv_out(ys, D - NINV, NINV, toks0)
    rh = jax.lax.broadcasted_iota(jnp.int32, (80, 128), 0)
    ch = jax.lax.broadcasted_iota(jnp.int32, (80, 128), 1) & 3
    kmask = jnp.logical_and(rh >= DH * ch, rh < DH * ch + DH)
    kvm = [jnp.where(kmask, acc_m[g], 0.0).astype(BF16) for g in range(NG)]
    zm = [_cat([acc_m[g][GR:GR + 8, :]] * 16).T for g in range(NG)]
    zlb = jnp.broadcast_to(jnp.sum(zl[...], axis=1, keepdims=True), (128, 128))
    kl_t = []
    for t in range(5):
        gl = _groups_of_tile(t, 0)
        wd = min(D, 128 * (t + 1)) - 128 * t
        rl = jax.lax.broadcasted_iota(jnp.int32, (16 * len(gl), wd), 0) + 16 * gl[0]
        cl = jax.lax.broadcasted_iota(jnp.int32, (16 * len(gl), wd), 1) + 128 * t
        hl_ = 4 * (rl >> 4) + (rl & 3)
        blk = jnp.where(jnp.logical_and(cl >= DH * hl_, cl < DH * hl_ + DH), acc_l[t], 0.0)
        parts = []
        if gl[0] > 0:
            parts.append(jnp.zeros((16 * gl[0], wd), F32))
        parts.append(blk)
        if gl[-1] < NG - 1:
            parts.append(jnp.zeros((16 * (NG - 1 - gl[-1]), wd), F32))
        kl_t.append(_pb(_cat(parts).T))
    kvl = _cat(kl_t)
    wfl = _nn(_up(wot[:, 256:D]), _up(kvl[128:D // 2]))
    lane_b = jax.lax.broadcasted_iota(jnp.int32, (D // 2, 128), 1)
    wrem = jnp.where(lane_b < 64, wot2[...], _pb(wfl))

    ostart = [sum(OCH[:i]) for i in range(len(OCH))]

    def out_copy(i, r0=0, r1=D):
        sl = pl.ds(ostart[i] * 128, OCH[i] * 128)
        return cp(7, ob.at[r0:r1, sl], o_hbm.at[r0:r1, sl])

    def attn_phi(n, toks):
        mains, lefts, done = [], [], []
        for g in range(NG):
            p = logits(lambda r: pq[r:r + 8, n * 128:(n + 1) * 128], g)
            if toks is not None:
                p[1] = jnp.where(never, toks[g], p[1])
            mx = _fold8(jnp.maximum, p)
            mn = _fold8(jnp.minimum, p)
            e = [jnp.exp2(t - mx) for t in p] + [jnp.exp2(mn - t) for t in p]
            rp = _rcp(_fold8(jnp.add, e[0:9]))
            rn = _rcp(_fold8(jnp.add, e[9:18]))
            z = [zm[g][i * 8:(i + 1) * 8] for i in range(16)] + [zlb[g * 16 + i * 8:g * 16 + i * 8 + 8] for i in range(2)]
            dp = functools.reduce(jnp.add, [e[i] * z[i] for i in range(9)])
            dn = functools.reduce(jnp.add, [e[i] * z[i] for i in range(9, 18)])
            dh = dp * rp + dn * rn
            rd = _rcp(dh + pltpu.roll(dh, 4, 0) + 1e-6)
            sp = rp * rd
            sn_ = rn * rd
            ph = [t * sp for t in e[0:9]] + [t * sn_ for t in e[9:18]]
            mains.append(_cat(ph[0:16]).astype(BF16))
            lefts += ph[16:18]
            done.append(pltpu.bitcast(sn_, U32))
        return mains, _pb(_cat(lefts)), done

    def attn_o(phi):
        mains, left, _ = phi
        om = _cat([_nn(kvm[g], mains[g])[0:GR] for g in range(NG)])
        ol = _cat([_nn(_up(kvl[72 * q:72 * (q + 1), 0:64]), _up(left[0:32])) for q in range(2)])
        return om, _cat([_pb(_cat([om[0:288] + ol, om[288:D]])), left[32:64]])

    def finish(n, ot, riders=None):
        br = _cat([_nn(_up(wrem[72 * q:72 * (q + 1)]), _up(ot[256:320])) for q in range(4)])
        w0 = wot[:, 0:128]
        if riders:
            blks = [w0[r:r + 8] for r in range(0, D // 2, 8)]
            for g in range(NG):
                blks[RID0 + RIDS * g] = jnp.where(never, riders[g], blks[RID0 + RIDS * g])
            w0 = _cat(blks)
        bt = _nn(_up(_cat([w0, wot[:, 128:512]], axis=1)), _up(ot[0:256])) + br
        gg = _cat([gs[:, n * 128:(n + 1) * 128]] * (D // 8))
        a = at[:, n * 128:(n + 1) * 128] * xb[:, n * 128:(n + 1) * 128].astype(F32)
        res = (bt + gg * (a - bt)).astype(BF16)
        if n == NB - 1:
            for r0, r1 in zip(LAST[:-1], LAST[1:]):
                ob[r0:r1, n * 128:(n + 1) * 128] = res[r0:r1]
                out_copy(len(OCH) - 1, r0, r1).start()
        else:
            ob[:, n * 128:(n + 1) * 128] = res
            for i in range(len(OCH)):
                if n + 1 == ostart[i] + OCH[i]:
                    out_copy(i).start()
        return br, bt

    nt0 = len(toks0)
    phi = {0: attn_phi(0, None),
           1: attn_phi(1, [toks0[(nt0 * g) // 16][0] for g in range(NG)]),
           2: attn_phi(2, [toks0[(nt0 * (g + 8)) // 16][0] for g in range(NG)])}
    om0, o0 = attn_o(phi[0])
    om1, o1 = attn_o(phi[1])
    ot = {0: o0, 1: o1}
    phi[3] = attn_phi(3, [om0[GR * g:GR * g + 8] for g in range(0, 8, 2)] + [om1[GR * g:GR * g + 8] for g in range(0, 8, 2)])
    for n in range(NB):
        br, bt = finish(n, ot[n], phi[n + RLAG][2] if n + RLAG < NB else None)
        if n + 2 < NB:
            om, ot[n + 2] = attn_o(phi[n + 2])
        if n + 4 < NB:
            tk = [br[0:8], bt[64:72], bt[208:216], bt[352:360], bt[496:504], om[0:8], om[4 * GR:4 * GR + 8], om[7 * GR + 64:7 * GR + 72]]
            phi[n + 4] = attn_phi(n + 4, tk)
    with _Scope('wait_out'):
        for i in range(len(OCH) - 1):
            out_copy(i).wait()
        for r0, r1 in zip(LAST[:-1], LAST[1:]):
            out_copy(len(OCH) - 1, r0, r1).wait()


@jax.jit
def pallas_gated_mix__ssm_conv_h3__linear_kernel_hedgehog__prompt_kernel(A_q, A_k, A_v, A_shift_k, A_ssm_k, A_ssm_D, B_x, B_wqkv, B_w_phi, B_wo, gate_w):
    fm, gm = _dft_consts()
    vm = pltpu.VMEM
    scratch = [
        vm((D, S), BF16), vm((D, S), BF16), vm((D, S), BF16), vm((D, S), BF16),
        vm((D, 3 * D), BF16), vm((D, D), BF16),
        vm((4, D), BF16), vm((D,), BF16), vm((D,), BF16), vm((DH, DH, H), BF16),
        vm((B, 2 * B), BF16), vm((2 * B, B), BF16),
        vm((MR // 2, D), U32), vm((D // 2, D), U32), vm((D // 2, 128), U32),
        vm((5, D, 128), F32), vm((2, GR, 640), F32), vm((D // 2, 640), U32),
        vm((D, S), F32), vm((KD, S), F32), vm((8, S), F32),
        vm((D, S), BF16), vm((C00 * 8, 2 * B), U32), vm((NINV * 8, 2 * B), U32),
        vm((8 * (CCS[0] + CCS[1]), 256), U32), vm((8 * CCS[2], 256), U32), vm((D + NB * 352, 256), U32),
        vm((NG * 64, SC), U32), vm((NG * 8, SC), U32),
        vm((NG * 40, SC), U32), vm((D // 2, SC), U32),
        vm((NG, 80, 128), F32), vm((48, D), F32), vm((128, 128), F32),
        pltpu.SemaphoreType.DMA((9,)),
    ]
    out_t = pl.pallas_call(
        _kernel,
        out_shape=jax.ShapeDtypeStruct((D, S), BF16),
        in_specs=[pl.BlockSpec(memory_space=pl.ANY)] * 12,
        out_specs=pl.BlockSpec(memory_space=pl.ANY),
        scratch_shapes=scratch,
        compiler_params=pltpu.CompilerParams(vmem_limit_bytes=100 * 1024 * 1024),
    )(A_q[0].T, A_k[0].T, A_v[0].T, A_shift_k.T, A_ssm_k, A_ssm_D, B_wqkv,
      jnp.transpose(B_w_phi, (1, 2, 0)), B_wo, gate_w, jnp.asarray(fm, BF16), jnp.asarray(gm, BF16))
    return out_t.T[None]
```

```python
import functools
import math

import jax
import jax.numpy as jnp
import numpy as np
import jax.experimental.pallas as pl
import jax.experimental.pallas.tpu as pltpu

S = 2048
D = 576
H = 32
DH = 18
NG = 8
GR = 72
B = 128
NB = S // B
NIT = 4
CCS = (64, 160, 176, 176)
COFF = tuple(sum(CCS[:i]) for i in range(NIT))
NINV = CCS[2]
C00 = D - 3 * NINV
SC = S // NIT
NT = SC // 128
KD = 544
MR = 2 * KD + D + 16
KO, VO, GO, QO = 0, KD, KD + D, KD + D + 16
LOG2E = math.log2(math.e)
F32 = jnp.float32
BF16 = jnp.bfloat16
U32 = jnp.uint32
OCH = (2, 2, 2, 2, 2, 2, 2, 1, 1)
LAST = (0, 384, 512, 576)
QC = 2
NOLM = 3
TRIM = 6
USKIP, CAP_U = 20, 24
CAP_R, CAP_K, CAP_V, CAP_I, CAP_RR = 50, 20, 44, 40, 36
TK0, TKS = 8, 56
OR0, ORS = 4, 1
RID0, RIDS, RLAG = 2, 3, 2


def _dft_consts():
    n = np.arange(B, dtype=np.float64)[:, None]
    k = np.arange(B, dtype=np.float64)[None, :]
    ang = 2.0 * np.pi * (2.0 * k + 0.5) * n / (2 * B)
    f = np.concatenate([np.cos(ang), -np.sin(ang)], axis=1)
    g = f.T / B
    return f.astype(np.float32), g.astype(np.float32)


def _nn(a, b):
    return jnp.dot(a, b, preferred_element_type=F32)


def _nt(a, b):
    return jax.lax.dot_general(a, b, (((1,), (1,)), ((), ())), preferred_element_type=F32)


def _pk(x):
    return pltpu.bitcast(x, U32)


def _up(x):
    return pltpu.bitcast(x, BF16)


def _cat(xs, axis=0):
    return xs[0] if len(xs) == 1 else jnp.concatenate(xs, axis=axis)


def _fold8(op, xs):
    r = functools.reduce(op, xs)
    return op(r, pltpu.roll(r, 4, 0))


def _rcp(x):
    return pl.reciprocal(x, approx=True)


def _groups_of_tile(t, off):
    lo = max(0, (128 * t - off) // GR)
    hi = min(NG - 1, (128 * t + 127 - off) // GR)
    return list(range(lo, hi + 1))


def _ds(start, size, align):
    if not isinstance(start, int):
        start = pl.multiple_of(start, align)
    return pl.ds(start, size)


def _kernel(x_hbm, k_hbm, v_hbm, sk_hbm, h_hbm, sd_hbm, w_hbm, wp_hbm, wo_hbm, gw_hbm, f_hbm, g_hbm,
            o_hbm,
            xb, kb, vb, hb, wb, wob, skb, sdb, gwb, wpb, fb, gb,
            wt, wot, wot2, cb, aps, emat, at, pq, gs, ob, ys0, ys, pkb0, pkb1, pkb2,
            phm, phl, vgp, vnp, kvam, kval, zl,
            sems):
    bump = [0, pkb0]

    def _pb(x):
        n = x.shape[0] // 2
        r, pkb = bump
        bump[0] += n
        pkb[r:r + n, 0:128] = _pk(x.astype(BF16))
        return pkb[r:r + n, 0:128]

    def get_never():
        return fb[0:16, 0:128].astype(F32)[0:8] > 2.0

    def cp(i, src, dst):
        return pltpu.make_async_copy(src, dst, sems.at[i])

    def step_copies(i, sem):
        rs = pl.ds(COFF[i], CCS[i])
        cs = pl.ds(i * SC, SC)
        return ([cp(sem[0], x_hbm.at[:, cs], xb.at[:, cs])],
                [cp(sem[1], s_.at[rs, :], d_.at[rs, :]) for s_, d_ in ((h_hbm, hb), (k_hbm, kb), (v_hbm, vb))])

    x0_, a0_ = step_copies(0, (3, 4))
    grp = [
        [cp(0, wp_hbm, wpb)],
        [cp(1, w_hbm.at[:, 768:1152], wb.at[:, 768:1152])],
        [cp(2, w_hbm.at[:, 384:768], wb.at[:, 384:768])],
        x0_ + [cp(3, sk_hbm, skb), cp(3, sd_hbm, sdb), cp(3, gw_hbm, gwb)],
        [cp(4, f_hbm, fb), cp(4, w_hbm.at[:, 1152:1728], wb.at[:, 1152:1728])] + a0_,
        sum(step_copies(1, (5, 5)), []) + [cp(5, g_hbm, gb), cp(5, wo_hbm, wob)],
        sum(step_copies(2, (6, 6)), []) + sum(step_copies(3, (6, 6)), []),
        [cp(8, w_hbm.at[:, 0:384], wb.at[:, 0:384])],
    ]
    for c in grp[0] + grp[1] + grp[3][1:] + grp[2] + grp[7] + grp[3][:1] + grp[4] + grp[5] + grp[6]:
        c.start()

    def wait(i):
        for c in grp[i]:
            c.wait()

    lane = jax.lax.broadcasted_iota(jnp.int32, (8, 128), 1)
    sub = jax.lax.broadcasted_iota(jnp.int32, (8, 128), 0)

    er = jax.lax.broadcasted_iota(jnp.int32, (D, 640), 0)
    ec = jax.lax.broadcasted_iota(jnp.int32, (D, 640), 1)
    emat[...] = _pk(jnp.where(ec == 64 + DH * (er & 31) + (er >> 5), 1.0, 0.0).astype(BF16))
    wait(0)
    tcat = _cat([wpb[d].astype(F32) for d in range(DH)], axis=1)
    amat = _nn(tcat.astype(BF16), _up(emat[...]))
    sub5 = jax.lax.broadcasted_iota(jnp.int32, (8, 640), 0)
    aps[1] = _cat([jnp.where(sub5 < 4, jnp.broadcast_to(amat[2 * fp:2 * fp + 1], (8, 640)),
                             jnp.broadcast_to(amat[2 * fp + 1:2 * fp + 2], (8, 640))) for fp in range(9)])

    def fold_mm(parts, which, off, t0, tiles):
        for t in tiles:
            gl = _groups_of_tile(t, off)
            a_t = aps[which, :, 128 * t:128 * (t + 1)]
            lhs = []
            for g in gl:
                lo = DH * (4 * g + (sub & 3)) + off - 128 * t
                msk = jnp.logical_and(lane >= lo, lane < lo + DH)
                lhs += [jnp.where(msk, a_t[fp * 8:fp * 8 + 8], 0.0) for fp in range(9)]
            r = _nt(_cat(lhs).astype(BF16), wb[:, 128 * (t0 + t):128 * (t0 + t + 1)])
            for i, g in enumerate(gl):
                piece = r[i * GR:(i + 1) * GR]
                parts[g] = piece if parts[g] is None else parts[g] + piece

    def fold_out(parts, ro, pairs):
        subd = jax.lax.broadcasted_iota(jnp.int32, (8, D), 0)
        out = []
        for p in pairs:
            us_, ds_ = [], []
            for g in (2 * p, 2 * p + 1):
                s0 = parts[g][0:8]
                r0 = jnp.where(subd < 4, s0, pltpu.roll(s0, 4, 0))
                us_.append(s0 - r0)
                ds_ += [parts[g][fp * 8:fp * 8 + 8] - r0 for fp in range(1, 9)]
            out += [pltpu.roll(us_[0], 4, 0) + us_[1]] + ds_
        r0 = (ro + 136 * pairs[0]) // 2
        wt[r0:r0 + 68 * len(pairs), :] = _pk((_cat(out) * LOG2E).astype(BF16))

    def logits(get, g):
        base = (g // 2) * 136
        x = get(base)
        if g % 2 == 0:
            x = pltpu.roll(x, 4, 0)
        return [jnp.where(sub < 4, 0.0, x)] + [get(base + 8 + (g % 2) * 64 + f * 8) for f in range(8)]

    def project(r0, r1, s0, toks=None, riders=None):
        xv = xb.at[:, _ds(s0, SC, 128)]
        lhs = wt[r0 // 2:r1 // 2, 512:D]
        if riders:
            never = get_never()[:, 0:64]
            riders = list(riders)
            blks = [lhs[r:r + 8] for r in range(0, (r1 - r0) // 2, 8)]
            for i in range(len(blks) - (len(riders) + 1) // 2, len(blks)):
                for _ in range(2):
                    if riders:
                        blks[i] = jnp.where(never, riders.pop(0)[:, 0:64], blks[i])
            lhs = _cat(blks)
        rr = _nn(_up(lhs), xv[512:D, :])
        if toks is not None:
            for r in range(0, r1 - r0, 16):
                toks.append((rr[r:r + 8, 0:128], CAP_R if riders is None else CAP_RR))

        def tile(n):
            pr = _nn(_up(wt[r0 // 2:r1 // 2, 0:512]), xv[0:512, n * 128:(n + 1) * 128]) + rr[:, n * 128:(n + 1) * 128]
            if toks is not None:
                for r in range(0, r1 - r0, 16):
                    toks.append((pr[r:r + 8], CAP_K if r0 + r < VO else CAP_V))
            return pr
        return tile

    def softmax_k(pk, n):
        lefts = []
        for g in range(NG):
            p = logits(lambda r: pk[r:r + 8], g)
            mx = _fold8(jnp.maximum, p)
            mn = _fold8(jnp.minimum, p)
            ep = [jnp.exp2(t - mx) for t in p]
            en = [jnp.exp2(mn - t) for t in p]
            rp = _rcp(_fold8(jnp.add, ep))
            rn = _rcp(_fold8(jnp.add, en))
            ph = [t * rp for t in ep] + [t * rn for t in en]
            phm[g * 64:(g + 1) * 64, n * 128:(n + 1) * 128] = _pk(_cat(ph[0:16]).astype(BF16))
            lefts += ph[16:18]
        left = _cat(lefts)
        phl[:, n * 128:(n + 1) * 128] = _pk(left.astype(BF16))
        return left

    def add_zl(lefts, first):
        tot = functools.reduce(jnp.add, lefts)
        zl[...] = tot if first else zl[...] + tot

    def pack_v(v, n):
        ones = jnp.ones((8, 128), F32)
        vgp[:, n * 128:(n + 1) * 128] = _pk(_cat(sum([[v[g * GR:(g + 1) * GR], ones] for g in range(NG)], [])).astype(BF16))
        vnp[:, n * 128:(n + 1) * 128] = _pk(v.astype(BF16))

    def kv_state(first):
        res_m, res_l = [], []
        for g in range(NG):
            r = _nt(_up(vgp[g * 40:(g + 1) * 40, :]), _up(phm[g * 64:(g + 1) * 64, :]))
            res_m.append(r if first else kvam[g] + r)
            kvam[g] = res_m[-1]
        for t in range(5):
            gl = _groups_of_tile(t, 0)
            hi = min(D, 128 * (t + 1))
            r = _nt(_up(phl[gl[0] * 8:(gl[-1] + 1) * 8, :]), _up(vnp[64 * t:hi // 2, :]))
            res_l.append(r if first else kval[0:16 * len(gl), 128 * t:hi] + r)
            kval[0:16 * len(gl), 128 * t:hi] = res_l[-1]
        return res_m, res_l

    def store_q(pr, off, sn):
        gs[:, _ds(sn, 128, 128)] = jax.nn.sigmoid(pr[off:off + 8])
        pq[:, _ds(sn, 128, 128)] = pr[off + 16:off + 16 + KD]

    def filter_spec(c0, nc):
        hv = hb.at[_ds(c0, nc, 16), :]
        dv = cb.at[4, _ds(c0, nc, 16), :]
        hl = _cat([hv[16 * cg:16 * cg + 16, m * B:(m + 1) * B] for cg in range(nc // 16) for m in range(NB)])
        hr = _nn(hl, fb[...])

        def spec(rg, m):
            r = (rg // 2) * 256 + m * 16 + (rg % 2) * 8
            cur = hr[r:r + 8]
            if m == 0:
                return cur[:, 0:B] + dv[rg * 8:rg * 8 + 8, :], cur[:, B:2 * B]
            return cur[:, 0:B], cur[:, B:2 * B]
        return [[spec(rg, m) for m in range(NB)] for rg in range(nc // 8)]

    def data_spec(c0, nc, toks):
        kv_ = kb.at[_ds(c0, nc, 16), :]
        vv_ = vb.at[_ds(c0, nc, 16), :]
        cv = cb.at[:, _ds(c0, nc, 16), :]
        kvs = []
        for rg in range(nc // 8):
            r = rg * 8
            co = [cv[t, r:r + 8, :] for t in range(4)]
            kf = kv_[r:r + 8, :].astype(F32)
            vf = vv_[r:r + 8, :].astype(F32)
            p1 = jnp.zeros((8, 128), F32)
            p2 = jnp.zeros((8, 128), F32)
            outs = []
            for j in range(NB):
                kj = kf[:, j * B:(j + 1) * B]
                r1 = pltpu.roll(kj, 1, 1)
                k1 = jnp.where(lane < 1, p1, r1)
                p1 = r1
                a = co[0] * kj + co[1] * k1
                b = co[2] * kj + co[3] * k1
                r2 = pltpu.roll(b, 2, 1)
                b2 = jnp.where(lane < 2, p2, r2)
                p2 = r2
                outs.append((a + b2) * vf[:, j * B:(j + 1) * B])
            kvs.append(_pb(_cat(outs)))
        ur = _nn(_up(_cat(kvs)), fb[...])
        for r in range(USKIP * 16, nc * NB, 16):
            toks.append((ur[r:r + 8, 0:B], CAP_U))
        return ur

    def mac_all(hs, ur, dest, nc, toks):
        never = get_never()
        nrg = nc // 8
        total = nrg * (136 * 8 + 80)
        cap = sum(c for _, c in toks)
        scale = total / cap
        st = {'i': 0, 'room': toks[0][1] * scale}

        def token(cost):
            while st['room'] < cost * 0.5 and st['i'] + 1 < len(toks):
                st['i'] += 1
                st['room'] += toks[st['i']][1] * scale
            st['room'] -= cost
            return toks[st['i']][0]

        for rg in range(nrg):
            prev = None
            for i0 in range(0, NB, 4):
                acc = [None] * 4
                for j in range(i0 + 4):
                    u_re = ur[rg * 128 + j * 8:rg * 128 + j * 8 + 8, 0:B]
                    u_im = ur[rg * 128 + j * 8:rg * 128 + j * 8 + 8, B:2 * B]
                    na = min(4, i0 + 4 - j)
                    tk_ = token(8 * na + 2)
                    u_re = jnp.where(never, tk_, u_re)
                    u_im = jnp.where(never, tk_, u_im)
                    for a in range(4):
                        m = i0 + a - j
                        if m < 0:
                            continue
                        h_re, h_im = hs[rg][m]
                        t_re = h_re * u_re - h_im * u_im
                        t_im = h_re * u_im + h_im * u_re
                        acc[a] = (t_re, t_im) if acc[a] is None else (acc[a][0] + t_re, acc[a][1] + t_im)
                out = []
                for a in range(4):
                    out.append(acc[a] if prev is None else (acc[a][0] - prev[1], acc[a][1] + prev[0]))
                    prev = acc[a]
                yv, slot = dest(rg)
                r0 = slot * 64 + i0 * 4
                yv[r0:r0 + 16, 0:B] = _pk(_cat([t[0] for t in out]).astype(BF16))
                yv[r0:r0 + 16, B:2 * B] = _pk(_cat([t[1] for t in out]).astype(BF16))

    def conv_out(yv, c0, nc, toks=None):
        hf = nc * 4
        av = at.at[_ds(c0, nc, 16), :]
        yr = _cat([_nn(_up(yv[0:hf]), gb[...]), _nn(_up(yv[hf:2 * hf]), gb[...])])
        if toks is not None:
            for r in range(0, 2 * hf, 16):
                toks.append((yr[r:r + 8], CAP_I))
        for rg in range(nc // 8):
            for i in range(NB):
                av[rg * 8:rg * 8 + 8, i * B:(i + 1) * B] = yr[rg * 128 + i * 8:rg * 128 + i * 8 + 8]

    pk_, pq_ = [None] * NG, [None] * NG
    wait(1)
    fold_mm(pk_, 1, 64, 4, (4, 3, 2))
    fold_out(pk_, KO, (2, 3))
    aps[0] = pltpu.roll(aps[1], 640 - 64, 1)
    wait(2)
    fold_mm(pk_, 1, 64, 4, (1, 0))
    fold_out(pk_, KO, (0, 1))
    fold_mm(pq_, 0, 0, 0, (4, 3))
    wait(7)
    fold_mm(pq_, 0, 0, 0, (2, 1, 0))
    fold_out(pq_, QO, (0, 1, 2, 3))

    wait(3)
    skf = skb[...].astype(F32)
    for t in range(4):
        cb[t] = jnp.broadcast_to(skf[t:t + 1, :], (128, D)).T
    cb[4] = jnp.broadcast_to(sdb[...].astype(F32).reshape(1, D), (128, D)).T
    wt[GO // 2:GO // 2 + 8, :] = _pk(jnp.broadcast_to(gwb[...].astype(F32).reshape(1, D), (16, D)).astype(BF16))
    tk = project(KO, KO + KD, 0)
    add_zl([softmax_k(tk(n), n) for n in range(NT)], True)
    toks = []
    tq = project(GO, MR, 0, toks)
    for n in range(QC):
        store_q(tq(n), 0, n * 128)

    wait(4)
    wt[VO // 2:(VO + D) // 2, :] = _pk(wb[:, 2 * D:3 * D].astype(F32).T.astype(BF16))
    store_q(tq(QC), 0, QC * 128)
    del toks[:]
    hs = filter_spec(0, CCS[0])
    ur = data_spec(0, CCS[0], toks)
    for n in range(QC + 1, NT):
        store_q(tq(n), 0, n * 128)
    tv = project(VO, VO + D, 0, toks)
    for n in range(NT):
        pack_v(tv(n), n)
    mac_all(hs, ur, lambda rg: (ys0, rg) if rg < C00 // 8 else (ys, rg - C00 // 8), CCS[0], toks[:-TRIM])

    def step(c0, nc, s0, ic0, inc, first):
        toks = []
        kv_state(first)
        hs = filter_spec(c0, nc)
        ur = data_spec(c0, nc, toks)
        riders = None
        if first:
            wot[...] = _pk(wob[...].astype(F32).T.astype(BF16))
            wot2[...] = jnp.zeros(wot2.shape, U32)
            wot2[:, 0:64] = wot[:, 512:D]
            riders = []
            for q in range(0, D // 2, 8):
                riders += [wot[q:q + 8, 128 * t:128 * (t + 1)] for t in range(4)] + [wot2[q:q + 8, :]]
        conv_out(ys0 if first else ys, ic0, inc, toks)
        tl = project(0, MR, s0, toks, riders)
        lefts = []
        for n in range(NT):
            pr = tl(n)
            lefts.append(softmax_k(pr, n))
            pack_v(pr[VO:VO + D], n)
            store_q(pr, GO, s0 + n * 128)
        add_zl(lefts, False)
        mac_all(hs, ur, lambda rg: (ys, rg + (NINV - nc) // 8), nc, toks[:-TRIM])

    wait(5)
    step(COFF[1], CCS[1], SC, 0, C00, True)
    wait(6)

    def loop_body(i, carry):
        bump[:] = [0, pkb1]
        step(COFF[2] + i * CCS[2], CCS[2], (2 + i) * SC, C00 + i * NINV, NINV, False)
        return carry

    jax.lax.fori_loop(0, 2, loop_body, 0)

    bump[:] = [0, pkb2]
    never = get_never()
    toks0 = []
    acc_m, acc_l = kv_state(False)
    conv_out(ys, D - NINV, NINV, toks0)
    rh = jax.lax.broadcasted_iota(jnp.int32, (80, 128), 0)
    ch = jax.lax.broadcasted_iota(jnp.int32, (80, 128), 1) & 3
    kmask = jnp.logical_and(rh >= DH * ch, rh < DH * ch + DH)
    kvm = [jnp.where(kmask, acc_m[g], 0.0).astype(BF16) for g in range(NG)]
    zm = [_cat([acc_m[g][GR:GR + 8, :]] * 16).T for g in range(NG)]
    zlb = jnp.broadcast_to(jnp.sum(zl[...], axis=1, keepdims=True), (128, 128))
    kl_t, kl_f = [], []
    for t in range(5):
        gl = _groups_of_tile(t, 0)
        wd = min(D, 128 * (t + 1)) - 128 * t
        rl = jax.lax.broadcasted_iota(jnp.int32, (16 * len(gl), wd), 0) + 16 * gl[0]
        cl = jax.lax.broadcasted_iota(jnp.int32, (16 * len(gl), wd), 1) + 128 * t
        hl_ = 4 * (rl >> 4) + (rl & 3)
        blk = jnp.where(jnp.logical_and(cl >= DH * hl_, cl < DH * hl_ + DH), acc_l[t], 0.0)
        parts = []
        if gl[0] > 0:
            parts.append(jnp.zeros((16 * gl[0], wd), F32))
        parts.append(blk)
        if gl[-1] < NG - 1:
            parts.append(jnp.zeros((16 * (NG - 1 - gl[-1]), wd), F32))
        kl_f.append(_cat(parts).T)
        kl_t.append(_pb(kl_f[-1]))
    kvl = _cat(kl_t)
    kvf = _cat(kl_f[0:3])
    coef = {}
    for g in range(4):
        for h4 in range(4):
            for v in range((DH * h4) // 8, (DH * h4 + DH - 1) // 8 + 1):
                for j in range(4):
                    k_ = 16 * g + 4 * j + h4
                    coef[g, h4, v, j] = jnp.broadcast_to(kvf[GR * g + 8 * v:GR * g + 8 * v + 8, k_:k_ + 1], (8, 128))
    wfl = _nn(_up(wot[:, 256:D]), _up(kvl[128:D // 2]))
    lane_b = jax.lax.broadcasted_iota(jnp.int32, (D // 2, 128), 1)
    wrem = jnp.where(lane_b < 64, wot2[...], _pb(wfl))

    ostart = [sum(OCH[:i]) for i in range(len(OCH))]

    def out_copy(i, r0=0, r1=D):
        sl = pl.ds(ostart[i] * 128, OCH[i] * 128)
        return cp(7, ob.at[r0:r1, sl], o_hbm.at[r0:r1, sl])

    def attn_phi(n, toks):
        mains, lefts, done = [], [], []
        g1 = 1.0 - gs[:, n * 128:(n + 1) * 128]
        for g in range(NG):
            p = logits(lambda r: pq[r:r + 8, n * 128:(n + 1) * 128], g)
            if toks is not None:
                p[1] = jnp.where(never, toks[g], p[1])
            mx = _fold8(jnp.maximum, p)
            mn = _fold8(jnp.minimum, p)
            e = [jnp.exp2(t - mx) for t in p] + [jnp.exp2(mn - t) for t in p]
            rp = _rcp(_fold8(jnp.add, e[0:9]))
            rn = _rcp(_fold8(jnp.add, e[9:18]))
            z = [zm[g][i * 8:(i + 1) * 8] for i in range(16)] + [zlb[g * 16 + i * 8:g * 16 + i * 8 + 8] for i in range(2)]
            dp = functools.reduce(jnp.add, [e[i] * z[i] for i in range(9)])
            dn = functools.reduce(jnp.add, [e[i] * z[i] for i in range(9, 18)])
            dh = dp * rp + dn * rn
            rd = _rcp(dh + pltpu.roll(dh, 4, 0) + 1e-6)
            rd = rd * g1
            sp = rp * rd
            sn_ = rn * rd
            ph = [t * sp for t in e[0:9]] + [t * sn_ for t in e[9:18]]
            mains.append(_cat(ph[0:16]).astype(BF16))
            lefts += ph[16:18]
            done.append(pltpu.bitcast(sn_, U32))
        return mains, (lefts[0:8], _pb(_cat(lefts[8:16]))), done, n

    def left_vpu(phi):
        lf = phi[1][0]
        rows = []
        for g in range(4):
            acc = [None] * 9
            for h4 in range(4):
                for j in range(4):
                    r_ = 4 * (j % 2) + h4
                    pb = jnp.broadcast_to(lf[2 * g + j // 2][r_:r_ + 1], (8, 128))
                    for v in range((DH * h4) // 8, (DH * h4 + DH - 1) // 8 + 1):
                        t = coef[g, h4, v, j] * pb
                        acc[v] = t if acc[v] is None else acc[v] + t
            rows += acc
        return rows

    def attn_o(phi, rows=None):
        mains, (lf, lp), _, n = phi
        om = _cat([_nn(kvm[g], mains[g])[0:GR] for g in range(NG)])
        if rows is None:
            lo = _pb(_cat(lf))
            ol = _cat([_nn(_up(kvl[72 * q:72 * (q + 1), 0:64]), _up(lo)) for q in range(2)])
        else:
            ol = _cat(rows)
        return om, _cat([_pb(_cat([om[0:288] + ol, om[288:D]])), lp])

    def finish(n, ot, riders=None, riders2=None):
        br = _cat([_nn(_up(wrem[72 * q:72 * (q + 1)]), _up(ot[256:320])) for q in range(4)])
        w0 = wot[:, 0:128]
        if riders:
            blks = [w0[r:r + 8] for r in range(0, D // 2, 8)]
            for g in range(NG):
                blks[RID0 + RIDS * g] = jnp.where(never, riders[g], blks[RID0 + RIDS * g])
            w0 = _cat(blks)
        w1 = wot[:, 128:256]
        if riders2 is not None:
            blks = [w1[r:r + 8] for r in range(0, D // 2, 8)]
            for i in range(36):
                p_ = min(35, OR0 + (ORS * i) // 4)
                blks[p_] = jnp.where(never, pltpu.bitcast(riders2[i], U32), blks[p_])
            w1 = _cat(blks)
        bt = _nn(_up(_cat([w0, w1, wot[:, 256:512]], axis=1)), _up(ot[0:256])) + br
        gg = _cat([gs[:, n * 128:(n + 1) * 128]] * (D // 8))
        a = at[:, n * 128:(n + 1) * 128] * xb[:, n * 128:(n + 1) * 128].astype(F32)
        res = (bt + gg * a).astype(BF16)
        if n == NB - 1:
            for r0, r1 in zip(LAST[:-1], LAST[1:]):
                ob[r0:r1, n * 128:(n + 1) * 128] = res[r0:r1]
                out_copy(len(OCH) - 1, r0, r1).start()
        else:
            ob[:, n * 128:(n + 1) * 128] = res
            for i in range(len(OCH)):
                if n + 1 == ostart[i] + OCH[i]:
                    out_copy(i).start()
        return br, bt

    nt0 = len(toks0)
    phi = {0: attn_phi(0, None),
           1: attn_phi(1, [toks0[(nt0 * g) // 16][0] for g in range(NG)]),
           2: attn_phi(2, [toks0[(nt0 * (g + 8)) // 16][0] for g in range(NG)])}
    om0, o0 = attn_o(phi[0])
    om1, o1 = attn_o(phi[1])
    ot = {0: o0, 1: o1}
    phi[3] = attn_phi(3, [om0[GR * g:GR * g + 8] for g in range(0, 8, 2)] + [om1[GR * g:GR * g + 8] for g in range(0, 8, 2)])
    for n in range(NB):
        rows = left_vpu(phi[n + 2]) if NOLM <= n + 2 < NB else None
        br, bt = finish(n, ot[n], phi[n + RLAG][2] if n + RLAG < NB else None, rows)
        if n + 2 < NB:
            om, ot[n + 2] = attn_o(phi[n + 2], rows)
        if n + 4 < NB:
            tk = [bt[TK0 + TKS * g:TK0 + TKS * g + 8] for g in range(NG)]
            phi[n + 4] = attn_phi(n + 4, tk)
    for i in range(len(OCH) - 1):
        out_copy(i).wait()
    for r0, r1 in zip(LAST[:-1], LAST[1:]):
        out_copy(len(OCH) - 1, r0, r1).wait()


@jax.jit
def pallas_gated_mix__ssm_conv_h3__linear_kernel_hedgehog__prompt_kernel(A_q, A_k, A_v, A_shift_k, A_ssm_k, A_ssm_D, B_x, B_wqkv, B_w_phi, B_wo, gate_w):
    fm, gm = _dft_consts()
    vm = pltpu.VMEM
    scratch = [
        vm((D, S), BF16), vm((D, S), BF16), vm((D, S), BF16), vm((D, S), BF16),
        vm((D, 3 * D), BF16), vm((D, D), BF16),
        vm((4, D), BF16), vm((D,), BF16), vm((D,), BF16), vm((DH, DH, H), BF16),
        vm((B, 2 * B), BF16), vm((2 * B, B), BF16),
        vm((MR // 2, D), U32), vm((D // 2, D), U32), vm((D // 2, 128), U32),
        vm((5, D, 128), F32), vm((2, GR, 640), F32), vm((D // 2, 640), U32),
        vm((D, S), F32), vm((KD, S), F32), vm((8, S), F32),
        vm((D, S), BF16), vm((C00 * 8, 2 * B), U32), vm((NINV * 8, 2 * B), U32),
        vm((8 * (CCS[0] + CCS[1]), 256), U32), vm((8 * CCS[2], 256), U32), vm((D + NB * 352, 256), U32),
        vm((NG * 64, SC), U32), vm((NG * 8, SC), U32),
        vm((NG * 40, SC), U32), vm((D // 2, SC), U32),
        vm((NG, 80, 128), F32), vm((48, D), F32), vm((128, 128), F32),
        pltpu.SemaphoreType.DMA((9,)),
    ]
    out_t = pl.pallas_call(
        _kernel,
        out_shape=jax.ShapeDtypeStruct((D, S), BF16),
        in_specs=[pl.BlockSpec(memory_space=pl.ANY)] * 12,
        out_specs=pl.BlockSpec(memory_space=pl.ANY),
        scratch_shapes=scratch,
        compiler_params=pltpu.CompilerParams(vmem_limit_bytes=100 * 1024 * 1024),
    )(A_q[0].T, A_k[0].T, A_v[0].T, A_shift_k.T, A_ssm_k, A_ssm_D, B_wqkv,
      jnp.transpose(B_w_phi, (1, 2, 0)), B_wo, gate_w, jnp.asarray(fm, BF16), jnp.asarray(gm, BF16))
    return out_t.T[None]
```
